```python
import jax
import jax.numpy as jnp

def _softmax(x, axis=-1):
    return jax.nn.softmax(x, axis=axis)

def _gelu(x):
    return jax.nn.gelu(x, approximate=True)

def _silu(x):
    return jax.nn.silu(x)

def _sigmoid(x):
    return jax.nn.sigmoid(x)

def _layernorm(x, axis=-1, eps=1e-05):
    m = jnp.mean(x, axis=axis, keepdims=True)
    v = jnp.var(x, axis=axis, keepdims=True)
    return (x - m) / jnp.sqrt(v + eps)

def _scatter_add(tgt, idx, src, axis=0):
    return tgt.at[idx].add(src)

def _segment_sum(src, seg, n):
    return jax.ops.segment_sum(src, seg, n)

class _Rng:

    def __init__(self, key):
        self._k = key

    def _next(self):
        self._k, sub = jax.random.split(self._k)
        return sub

    def normal(self, shape):
        return jax.random.normal(self._next(), shape, dtype=jnp.bfloat16)

    def randint(self, lo, hi, shape):
        return jax.random.randint(self._next(), shape, lo, hi, dtype=jnp.int32)

    def uniform(self, shape, lo=0.0, hi=1.0):
        return jax.random.uniform(self._next(), shape, jnp.bfloat16, lo, hi)

    def permutation(self, n):
        return jax.random.permutation(self._next(), n)
kernel_name = 'concat_heads__memory_aug_recurrent_mem_tr__spectral_gfnet__prompt'

def setup_inputs():
    _rng = _Rng(jax.random.key(int.from_bytes(__import__("os").urandom(4), "little")))
    _w = lambda a: (lambda t: t.astype(jnp.bfloat16) if jnp.issubdtype(t.dtype, jnp.floating) else t)(jnp.asarray(a))

    def _A_setup():
        B, S, Dm = (1, 2048, 1024)
        H, Dh = (32, 128)
        M, seg = (8, 32)
        seg = min(seg, S)
        S = S // seg * seg
        return {'x': _w((lambda *s: _rng.normal(s) * 0.05)(B, S, Dm)), 'mem0': _w((lambda *s: _rng.normal(s) * 0.05)(B, M, Dm)), 'Wq': _w((lambda *s: _rng.normal(s) * 0.05)(Dm, H, Dh) * Dm ** (-0.5)), 'Wk': _w((lambda *s: _rng.normal(s) * 0.05)(Dm, H, Dh) * Dm ** (-0.5)), 'Wv': _w((lambda *s: _rng.normal(s) * 0.05)(Dm, H, Dh) * Dm ** (-0.5)), 'Wo': _w((lambda *s: _rng.normal(s) * 0.05)(H, Dh, Dm) * (H * Dh) ** (-0.5)), 'seg_len': seg}
    _A_in = _A_setup()

    def _B_setup():
        B, S, D = (1, 2048, 1024)
        Df = D // 2 + 1
        return {'x': _w((lambda *s: _rng.normal(s) * 0.05)(B, S, D)), 'w_r': _w((lambda *s: _rng.normal(s) * 0.05)(S, Df) * 0.02), 'w_i': _w((lambda *s: _rng.normal(s) * 0.05)(S, Df) * 0.02)}
    _B_in = _B_setup()
    return {'A_x': _A_in['x'], 'A_mem0': _A_in['mem0'], 'A_Wq': _A_in['Wq'], 'A_Wk': _A_in['Wk'], 'A_Wv': _A_in['Wv'], 'A_Wo': _A_in['Wo'], 'A_seg_len': _A_in['seg_len'], 'B_x': _B_in['x'], 'B_w_r': _B_in['w_r'], 'B_w_i': _B_in['w_i']}

def reference(A_x, A_mem0, A_Wq, A_Wk, A_Wv, A_Wo, A_seg_len, B_x, B_w_r, B_w_i):

    def _A_ref(x, mem0, Wq, Wk, Wv, Wo, seg_len):
        B, S, Dm = x.shape
        H, Dh = (Wq.shape[1], Wq.shape[2])
        M = mem0.shape[1]
        scale = Dh ** (-0.5)
        n_seg = S // seg_len
        L = M + seg_len
        idx = jnp.arange(L)
        mask = (idx[:, None] < M) | (idx[:, None] >= idx[None, :])
        mem = mem0
        outs = []
        for s in range(n_seg):
            xs = x[:, s * seg_len:(s + 1) * seg_len, :].copy()
            h = jnp.concatenate([mem, xs], axis=1)
            q = jnp.einsum('btd,dhe->bhte', h, Wq)
            k = jnp.einsum('btd,dhe->bhte', h, Wk)
            v = jnp.einsum('btd,dhe->bhte', h, Wv)
            scores = jnp.einsum('bhqe,bhke->bhqk', q, k) * scale
            scores = jnp.where(mask[None, None], scores, -1000000000.0)
            p = _softmax(scores, axis=-1)
            o = jnp.einsum('bhqk,bhke->bhqe', p, v)
            o = jnp.einsum('bhte,hed->btd', o, Wo)
            mem = o[:, :M, :].copy()
            outs.append(o[:, M:, :])
        return jnp.concatenate(outs, axis=1)

    def _B_ref(x, w_r, w_i):
        B, S, D = x.shape
        X = (lambda x, axes=(-2, -1): jnp.fft.rfft2(x.astype(jnp.float32), axes=axes))(x, axes=(-2, -1))
        W = w_r + 1j * w_i
        X = X * W
        y = (lambda x, s, axes=(-2, -1): jnp.fft.irfft2(x, s=s, axes=axes).astype(jnp.bfloat16))(X, (S, D), axes=(-2, -1))
        return y
    a = _A_ref(A_x, A_mem0, A_Wq, A_Wk, A_Wv, A_Wo, A_seg_len)
    b = _B_ref(B_x, B_w_r, B_w_i)
    return jnp.concatenate([a, b], axis=-1)
```

```python
import numpy as np

import jax
import jax.numpy as jnp
from jax import lax
import jax.experimental.pallas as pl
import jax.experimental.pallas.tpu as pltpu

F32 = jnp.float32
BF16 = jnp.bfloat16
U32 = jnp.uint32

_S = 2048
_D = 1024
_H = 32
_M = 8
_SEG = 32
_L = _M + _SEG
_NSEG = _S // _SEG
_KR = 520
_RES = (1, 7, 2, 6, 3, 5, 4, 0)

_NT = (((1,), (1,)), ((), ()))


def _dft_constants():
    b = np.arange(128)

    def cs(k):
        ang = -2.0 * np.pi * ((k[:, None] * b[None, :]) % _D) / _D
        return np.cos(ang), np.sin(ang)

    j = np.arange(64)
    fd = np.zeros((1040, 256))
    for g, r in enumerate((1, 2, 3)):
        c1, s1 = cs(r + 8 * j)
        c2, s2 = cs(8 - r + 8 * j)
        fd[g * 256:(g + 1) * 256] = np.block([[c1, -s1], [c2, s2], [s1, c1], [s2, -c2]])
    c4, s4 = cs(4 + 8 * j)
    fd[768:896, :128] = np.concatenate([c4, s4], 0)
    c0, s0 = cs(8 * np.arange(72))
    c0[65:] = 0.0
    s0[64:] = 0.0
    s0[0] = 0.0
    fd[768:896, 128:] = np.concatenate([c0[:64], s0[:64]], 0)
    c0[0] *= 0.5
    c0[64] *= 0.5
    fd[896:1040, :128] = np.concatenate([c0, s0], 0)

    cm = []
    for a in range(16):
        ang = -2.0 * np.pi * (((16 * b + a)[:, None] * b[None, :]) % _S) / _S
        c, s = np.cos(ang), np.sin(ang)
        cm.append(np.block([[c, s], [-s, c]]))
    cm = np.stack(cm) * np.sqrt(2.0 / (_S * _D))
    return tuple(np.asarray(v, np.float32).astype(BF16) for v in (fd, cm))


_CONSTS = _dft_constants()


def _dft4(x, sign):
    (ar, ai), (br, bi), (cr, ci), (dr, di) = x
    t0r, t0i, t1r, t1i = ar + cr, ai + ci, ar - cr, ai - ci
    t2r, t2i, t3r, t3i = br + dr, bi + di, br - dr, bi - di
    lo = (t1r + t3i, t1i - t3r)
    hi = (t1r - t3i, t1i + t3r)
    if sign > 0:
        lo, hi = hi, lo
    return [(t0r + t2r, t0i + t2i), lo, (t0r - t2r, t0i - t2i), hi]


def _twiddle16(z, e, sign):
    zr, zi = z
    if e == 0:
        return z
    if e == 4:
        return (-zi, zr) if sign > 0 else (zi, -zr)
    h = float(np.sqrt(0.5))
    if e == 2:
        return ((zr - zi) * h, (zr + zi) * h) if sign > 0 else ((zr + zi) * h, (zi - zr) * h)
    if e == 6:
        return ((zr + zi) * -h, (zr - zi) * h) if sign > 0 else ((zi - zr) * h, (zr + zi) * -h)
    c = float(np.cos(2 * np.pi * e / 16))
    s = float(sign * np.sin(2 * np.pi * e / 16))
    return (zr * c - zi * s, zr * s + zi * c)


def _dft16(x, sign):
    cols = [_dft4([x[n1 + 4 * n2] for n2 in range(4)], sign) for n1 in range(4)]
    out = [None] * 16
    for k2 in range(4):
        res = _dft4([_twiddle16(cols[n1][k2], n1 * k2, sign) for n1 in range(4)], sign)
        for k1 in range(4):
            out[k2 + 4 * k1] = res[k1]
    return out


def _kernel(ax_hbm, mem_ref, wq_hbm, wk_hbm, wv_hbm, wo_hbm, bx_hbm, wr_hbm, wi_hbm,
            wrn_ref, win_ref, fd_hbm, cm_hbm, out_hbm,
            wqkv, wo, ax, ao, bx, wr, wi, fd, cm, y, h_ref, ob_ref, acc_ref,
            sem_w, sem_m, sem_o):
    qkv_u32 = [w.bitcast(U32) for w in (wq_hbm, wk_hbm, wv_hbm)]
    wo_u32 = wo_hbm.bitcast(U32)
    bx_u32 = bx_hbm.bitcast(U32)
    out_u32 = out_hbm.bitcast(U32)
    cp_bx = [pltpu.make_async_copy(bx_u32.at[:, c, :], bx.at[c], sem_m.at[6 + c])
             for c in range(8)]
    cp_fd = pltpu.make_async_copy(fd_hbm, fd, sem_m.at[0])
    cp_cm = pltpu.make_async_copy(cm_hbm, cm, sem_m.at[1])
    cp_w = [pltpu.make_async_copy(
        src.at[pl.ds(0, 512)].bitcast(U32).at[:, pl.ds(m1 * 128, 128)], dst.at[m1], sem_m.at[2])
        for src, dst in ((wr_hbm, wr), (wi_hbm, wi)) for m1 in range(16)]
    cp_qkv = [pltpu.make_async_copy(qkv_u32[j].at[:, hp, :], wqkv.at[j * 16 + hp + 1],
                                    sem_w.at[j * 16 + hp])
              for j in range(3) for hp in range(16)]
    cp_wo = [pltpu.make_async_copy(wo_u32.at[:, pl.ds(n * 128, 128)], wo.at[n], sem_m.at[3])
             for n in range(8)]
    cp_ax0 = pltpu.make_async_copy(ax_hbm.at[pl.ds(0, 256)], ax.at[pl.ds(0, 256)], sem_m.at[4])
    cp_ax1 = pltpu.make_async_copy(ax_hbm.at[pl.ds(256, _S - 256)], ax.at[pl.ds(256, _S - 256)],
                                   sem_m.at[5])
    cp_fd.start()
    cp_bx[0].start()
    cp_cm.start()
    for c in cp_bx[1:]:
        c.start()
    for c in cp_w:
        c.start()
    cp_fd.wait()
    cp_cm.wait()
    for c in cp_qkv:
        c.start()
    cp_ax0.start()
    for c in cp_wo:
        c.start()
    cp_ax1.start()

    h2 = float(np.sqrt(0.5))

    def half(u, par):
        u = (u << 16) if par == 0 else (u & jnp.uint32(0xFFFF0000))
        return lax.bitcast_convert_type(u, F32)

    def forward(c, carry):
        pltpu.make_async_copy(bx_u32.at[:, c, :], bx.at[c], sem_m.at[6 + c]).wait()
        for par in range(2):
            a = 2 * c + par
            x = [half(bx[c, :, t * 128:(t + 1) * 128], par) for t in range(8)]
            e0, e1, e2, e3 = x[0] + x[4], x[0] - x[4], x[2] + x[6], x[2] - x[6]
            o0, o1, o2, o3 = x[1] + x[5], x[1] - x[5], x[3] + x[7], x[3] - x[7]
            ee, oo = e0 + e2, o0 + o2
            p, q = (o1 - o3) * h2, (o1 + o3) * h2
            ts = ((e1 + p, -(e3 + q)), (e0 - e2, o2 - o0), (e1 - p, e3 - q))
            re, im = [], []
            for g in range(3):
                t = jnp.concatenate([ts[g][0].astype(BF16), ts[g][1].astype(BF16)], axis=1)
                r = lax.dot_general(fd[g * 256:(g + 1) * 256, :], t, _NT,
                                    preferred_element_type=F32)
                re.append(r[0:128])
                im.append(r[128:256])
            r = lax.dot_general(fd[768:896, 0:128], (ee - oo).astype(BF16), _NT,
                                preferred_element_type=F32)
            re.append(r[0:64])
            im.append(r[64:128])
            r = lax.dot_general(fd[896:1040, 0:128], (ee + oo).astype(BF16), _NT,
                                preferred_element_type=F32)
            re.append(r[0:72])
            im.append(r[72:144])
            for r0, r1, g0, g1 in ((0, 256, 0, 2), (256, _KR, 2, 5)):
                u = jnp.concatenate([jnp.concatenate(re[g0:g1], axis=0),
                                     jnp.concatenate(im[g0:g1], axis=0)], axis=1)
                y[a, r0:r1, :] = jnp.dot(u, cm[a], preferred_element_type=F32)
        return carry

    lax.fori_loop(0, 8, forward, 0)
    for c in cp_w:
        c.wait()

    def spectral(rows, filt):
        xf = _dft16([(y[a, rows, 0:128], y[a, rows, 128:256]) for a in range(16)], -1)
        v = []
        for m1 in range(16):
            (xr, xi), (fr, fi) = xf[m1], filt(m1)
            v.append((xr * fr - xi * fi, xr * fi + xi * fr))
        res = _dft16(v, +1)
        for a in range(16):
            y[a, rows, 0:128] = res[a][0]
            y[a, rows, 128:256] = res[a][1]

    def spectral_pair(i, carry):
        c, jg = i // 8, i % 8
        w_rows = pl.ds(jg * 32 + c, 8, stride=4)
        for par in range(2):
            blk = _RES.index(par)
            for cc in range(1, 4):
                blk = jnp.where(c == cc, _RES.index(2 * cc + par), blk)
            spectral(pl.ds(pl.multiple_of(blk * 64 + jg * 8, 8), 8),
                     lambda m1: (half(wr[m1, w_rows, :], par), half(wi[m1, w_rows, :], par)))
        return carry

    lax.fori_loop(0, 32, spectral_pair, 0)
    spectral(pl.ds(512, 8),
             lambda m1: tuple(jnp.broadcast_to(w[0:1, m1 * 128:(m1 + 1) * 128].astype(F32), (8, 128))
                             for w in (wrn_ref, win_ref)))

    sign = jnp.where(lax.broadcasted_iota(jnp.int32, (128, 256), 0) % 2 == 0, 1.0, -1.0)

    def b_out_copy(c):
        return pltpu.make_async_copy(bx.at[c], out_u32.at[:, c, pl.ds(_D, _D)], sem_o.at[0])

    def inverse(c, carry):
        outs = []
        for par in range(2):
            a = 2 * c + par
            qs = []
            for g in range(3):
                z = lax.dot_general(cm[a], y[a, g * 128:(g + 1) * 128, :].astype(BF16), _NT,
                                    preferred_element_type=F32)
                r = jnp.dot(jnp.concatenate([z[0:128], z[128:256]], axis=1),
                            fd[g * 256:(g + 1) * 256, :], preferred_element_type=F32)
                qs.append((r[:, 0:128], r[:, 128:256]))
            (q1r, q1i), (q2r, q2i), (q3r, q3i) = qs
            z = lax.dot_general(cm[a], y[a, 384:512, :].astype(BF16), _NT,
                                preferred_element_type=F32)
            zr, zi = z[0:128], z[128:256]
            low = lax.broadcasted_iota(jnp.int32, (128, 128), 1) < 64
            r4 = jnp.dot(jnp.where(low, zr, pltpu.roll(zi, 64, 1)), fd[768:896, 0:128],
                         preferred_element_type=F32)
            r0 = jnp.dot(jnp.where(low, pltpu.roll(zr, 64, 1), zi), fd[768:896, 128:256],
                         preferred_element_type=F32)
            r0 = r0 + lax.dot_general(cm[a, 0:128, :], (y[a, 512:513, :] * sign).astype(BF16),
                                      _NT, preferred_element_type=F32)
            ee, oo = r0 + r4, r0 - r4
            e0, e2, o0, o2 = ee + q2r, ee - q2r, oo - q2i, oo + q2i
            e1, e3 = q1r + q3r, q3i - q1i
            p, q = (q1r - q3r) * h2, (q1i + q3i) * h2
            o1, o3 = p - q, -(p + q)
            cols = (e0 + e1, o0 + o1, e2 + e3, o2 + o3, e0 - e1, o0 - o1, e2 - e3, o2 - o3)
            outs.append([lax.bitcast_convert_type(v.astype(BF16).astype(F32), U32)
                         for v in cols])
        for t in range(8):
            bx[c, :, t * 128:(t + 1) * 128] = (outs[0][t] >> 16) | outs[1][t]
        b_out_copy(c).start()
        return carry

    lax.fori_loop(0, 8, inverse, 0)

    for i in range(48):
        cp_qkv[i].wait()

        def repack(g, carry, i=i):
            src = pl.multiple_of(g * 128, 128)
            dst = pl.multiple_of(g * 64, 64)
            ev = wqkv[i + 1, pl.ds(src, 64, stride=2), :]
            od = wqkv[i + 1, pl.ds(src + 1, 64, stride=2), :]
            wqkv[i, pl.ds(dst, 64), :] = (ev & jnp.uint32(0xFFFF)) | (od << 16)
            wqkv[i, pl.ds(512 + dst, 64), :] = (ev >> 16) | (od & jnp.uint32(0xFFFF0000))
            return carry

        lax.fori_loop(0, 8, repack, 0, unroll=True)

    cp_ax0.wait()
    for c in cp_wo:
        c.wait()

    qi = lax.broadcasted_iota(jnp.int32, (_L, _L), 0)
    ki = lax.broadcasted_iota(jnp.int32, (_L, _L), 1)
    mask = (qi < _M) | (qi >= ki)
    scale = 128 ** -0.5
    group = 4
    n_group = _H // group

    h_ref[0:_M, :] = mem_ref[...].astype(F32)
    h_ref[_M:_L, :] = ax[0:_SEG, :].astype(F32)

    def a_out_copy(s):
        rows = pl.ds(2 * s, 2)
        return pltpu.make_async_copy(ao.at[rows], out_hbm.at[rows, :, pl.ds(0, _D)],
                                     sem_o.at[1])

    def step(s, carry):
        @pl.when(s == 6)
        def _():
            cp_ax1.wait()

        st = {}

        def proj(j, hd):
            w = wqkv[j * 16 + hd // 2, (hd % 2) * 512:(hd % 2 + 1) * 512, :]
            st[j, hd] = jnp.dot(h_ref[...], pltpu.bitcast(w, BF16), preferred_element_type=F32)

        def scores(hd):
            sc = lax.dot_general(st[0, hd], st[1, hd], _NT, preferred_element_type=F32) * scale
            sc = jnp.where(mask, sc, -1000000000.0)
            p = jnp.exp(sc - jnp.max(sc, axis=1, keepdims=True))
            st['p', hd] = p
            st['l', hd] = 1.0 / jnp.sum(p, axis=1, keepdims=True)

        def pv(hd):
            o = jnp.dot(st['p', hd], st[2, hd], preferred_element_type=F32)
            ob_ref[:, hd * 128:(hd + 1) * 128] = o * st['l', hd]

        def w_out(g, n):
            lanes = slice(n * 128, (n + 1) * 128)
            w = wo[n, g * group * 64:(g + 1) * group * 64, :]
            r = jnp.dot(ob_ref[:, g * group * 128:(g + 1) * group * 128],
                        pltpu.bitcast(w, BF16), preferred_element_type=F32)
            if g > 0:
                r = r + acc_ref[:, lanes]
            if g < n_group - 1:
                acc_ref[:, lanes] = r
            else:
                h_ref[0:_M, lanes] = r[0:_M].astype(BF16).astype(F32)
                ao[2 * s, :, lanes] = r[_M:_M + 16].astype(BF16)
                ao[2 * s + 1, :, lanes] = r[_M + 16:_L].astype(BF16)

        def next_x():
            nxt = jnp.minimum(s + 1, _NSEG - 1)
            h_ref[_M:_L, :] = ax[pl.ds(pl.multiple_of(nxt * _SEG, _SEG), _SEG), :].astype(F32)

        ops, pending = [], []
        for hd in range(_H):
            ops.append((proj, 0, hd))
            if hd >= 1:
                ops.append((scores, hd - 1))
            ops.append((proj, 1, hd))
            for _ in range(8 // group):
                if pending:
                    ops.append(pending.pop(0))
            ops.append((proj, 2, hd))
            if hd >= 1:
                ops.append((pv, hd - 1))
                if (hd - 1) % group == group - 1:
                    pending += [(w_out, (hd - 1) // group, n) for n in range(8)]
        ops.append((next_x,))
        ops.append((scores, _H - 1))
        ops += pending
        ops.append((pv, _H - 1))
        ops += [(w_out, n_group - 1, n) for n in range(8)]
        for op in ops:
            op[0](*op[1:])
        a_out_copy(s).start()
        return carry

    lax.fori_loop(0, _NSEG, step, 0)

    def drain_b(a, carry):
        b_out_copy(a).wait()
        return carry

    def drain_a(s, carry):
        a_out_copy(s).wait()
        return carry

    lax.fori_loop(0, 8, drain_b, 0)
    lax.fori_loop(0, _NSEG, drain_a, 0)


@jax.jit
def _run(A_x, A_mem0, A_Wq, A_Wk, A_Wv, A_Wo, B_x, B_w_r, B_w_i):
    hbm = pl.BlockSpec(memory_space=pltpu.HBM)
    vmem = pl.BlockSpec(memory_space=pltpu.VMEM)
    nyquist = pl.BlockSpec((16, _S), lambda i: (512 // 16, 0))
    wr, wi = B_w_r.T, B_w_i.T
    out = pl.pallas_call(
        _kernel,
        grid=(1,),
        out_shape=jax.ShapeDtypeStruct((128, 16, 2 * _D), BF16),
        in_specs=[hbm, vmem, hbm, hbm, hbm, hbm, hbm, hbm, hbm, nyquist, nyquist, hbm, hbm],
        out_specs=hbm,
        scratch_shapes=[
            pltpu.VMEM((49, 1024, 128), U32),
            pltpu.VMEM((8, 2048, 128), U32),
            pltpu.VMEM((_S, _D), BF16),
            pltpu.VMEM((128, 16, _D), BF16),
            pltpu.VMEM((8, 128, _D), U32),
            pltpu.VMEM((16, 256, 128), U32),
            pltpu.VMEM((16, 256, 128), U32),
            pltpu.VMEM((1040, 256), BF16),
            pltpu.VMEM((16, 256, 256), BF16),
            pltpu.VMEM((16, _KR, 256), F32),
            pltpu.VMEM((_L, _D), F32),
            pltpu.VMEM((_L, _H * 128), F32),
            pltpu.VMEM((_L, _D), F32),
            pltpu.SemaphoreType.DMA((48,)),
            pltpu.SemaphoreType.DMA((14,)),
            pltpu.SemaphoreType.DMA((2,)),
        ],
        compiler_params=pltpu.CompilerParams(vmem_limit_bytes=100 * 1024 * 1024),
    )(A_x.reshape(_S, _D), A_mem0.reshape(_M, _D), A_Wq, A_Wk, A_Wv,
      A_Wo.reshape(_H * 128, _D), B_x.reshape(128, 16, _D), wr, wi, wr, wi, *_CONSTS)
    return out.reshape(1, _S, 2 * _D)


def pallas_concat_heads__memory_aug_recurrent_mem_tr__spectral_gfnet__prompt_kernel(
    A_x, A_mem0, A_Wq, A_Wk, A_Wv, A_Wo, A_seg_len, B_x, B_w_r, B_w_i,
):
    assert int(A_seg_len) == _SEG
    return _run(A_x, A_mem0, A_Wq, A_Wk, A_Wv, A_Wo, B_x, B_w_r, B_w_i)
```

```python
import numpy as np

import jax
import jax.numpy as jnp
from jax import lax
import jax.experimental.pallas as pl
import jax.experimental.pallas.tpu as pltpu

F32 = jnp.float32
BF16 = jnp.bfloat16
U32 = jnp.uint32

_S = 2048
_D = 1024
_H = 32
_M = 8
_SEG = 32
_L = _M + _SEG
_NSEG = _S // _SEG
_KR = 520
_RES = (1, 7, 2, 6, 3, 5, 4, 0)

_NT = (((1,), (1,)), ((), ()))


def _dft_constants():
    b = np.arange(128)

    def cs(k):
        ang = -2.0 * np.pi * ((k[:, None] * b[None, :]) % _D) / _D
        return np.cos(ang), np.sin(ang)

    j = np.arange(64)
    fd = np.zeros((1040, 256))
    for g, r in enumerate((1, 2, 3)):
        c1, s1 = cs(r + 8 * j)
        c2, s2 = cs(8 - r + 8 * j)
        fd[g * 256:(g + 1) * 256] = np.block([[c1, -s1], [c2, s2], [s1, c1], [s2, -c2]])
    c4, s4 = cs(4 + 8 * j)
    fd[768:896, :128] = np.concatenate([c4, s4], 0)
    c0, s0 = cs(8 * np.arange(72))
    c0[65:] = 0.0
    s0[64:] = 0.0
    s0[0] = 0.0
    fd[768:896, 128:] = np.concatenate([c0[:64], s0[:64]], 0)
    c0[0] *= 0.5
    c0[64] *= 0.5
    fd[896:1040, :128] = np.concatenate([c0, s0], 0)

    cm = []
    for a in range(16):
        ang = -2.0 * np.pi * (((16 * b + a)[:, None] * b[None, :]) % _S) / _S
        c, s = np.cos(ang), np.sin(ang)
        cm.append(np.block([[c, s], [-s, c]]))
    cm = np.stack(cm) * np.sqrt(2.0 / (_S * _D))
    return tuple(np.asarray(v, np.float32).astype(BF16) for v in (fd, cm))


_CONSTS = _dft_constants()


def _dft4(x, sign):
    (ar, ai), (br, bi), (cr, ci), (dr, di) = x
    t0r, t0i, t1r, t1i = ar + cr, ai + ci, ar - cr, ai - ci
    t2r, t2i, t3r, t3i = br + dr, bi + di, br - dr, bi - di
    lo = (t1r + t3i, t1i - t3r)
    hi = (t1r - t3i, t1i + t3r)
    if sign > 0:
        lo, hi = hi, lo
    return [(t0r + t2r, t0i + t2i), lo, (t0r - t2r, t0i - t2i), hi]


def _twiddle16(z, e, sign):
    zr, zi = z
    if e == 0:
        return z
    if e == 4:
        return (-zi, zr) if sign > 0 else (zi, -zr)
    h = float(np.sqrt(0.5))
    if e == 2:
        return ((zr - zi) * h, (zr + zi) * h) if sign > 0 else ((zr + zi) * h, (zi - zr) * h)
    if e == 6:
        return ((zr + zi) * -h, (zr - zi) * h) if sign > 0 else ((zi - zr) * h, (zr + zi) * -h)
    c = float(np.cos(2 * np.pi * e / 16))
    s = float(sign * np.sin(2 * np.pi * e / 16))
    return (zr * c - zi * s, zr * s + zi * c)


def _dft16(x, sign):
    cols = [_dft4([x[n1 + 4 * n2] for n2 in range(4)], sign) for n1 in range(4)]
    out = [None] * 16
    for k2 in range(4):
        res = _dft4([_twiddle16(cols[n1][k2], n1 * k2, sign) for n1 in range(4)], sign)
        for k1 in range(4):
            out[k2 + 4 * k1] = res[k1]
    return out


def _kernel(ax_hbm, mem_ref, wq_hbm, wk_hbm, wv_hbm, wo_hbm, bx_hbm, wr_hbm, wi_hbm,
            wrn_ref, win_ref, fd_hbm, cm_hbm, out_hbm,
            wqkv, wo, ax, ao, bx, wr, wi, fd, cm, y, h_ref, ob_ref, acc_ref,
            sem_w, sem_m, sem_o):
    qkv_u32 = [w.bitcast(U32) for w in (wq_hbm, wk_hbm, wv_hbm)]
    wo_u32 = wo_hbm.bitcast(U32)
    bx_u32 = bx_hbm.bitcast(U32)
    out_u32 = out_hbm.bitcast(U32)
    cp_bx = [pltpu.make_async_copy(bx_u32.at[:, c, :], bx.at[c], sem_m.at[6 + c])
             for c in range(8)]
    cp_fd = pltpu.make_async_copy(fd_hbm, fd, sem_m.at[0])
    cp_cm = pltpu.make_async_copy(cm_hbm, cm, sem_m.at[1])
    cp_w = [pltpu.make_async_copy(
        src.at[pl.ds(0, 512)].bitcast(U32).at[:, pl.ds(m1 * 128, 128)], dst.at[m1], sem_m.at[2])
        for src, dst in ((wr_hbm, wr), (wi_hbm, wi)) for m1 in range(16)]
    cp_qkv = [pltpu.make_async_copy(qkv_u32[j].at[:, hp, :], wqkv.at[j * 16 + hp + 1],
                                    sem_w.at[j * 16 + hp])
              for j in range(3) for hp in range(16)]
    cp_wo = [pltpu.make_async_copy(wo_u32.at[:, pl.ds(n * 128, 128)], wo.at[n], sem_m.at[3])
             for n in range(8)]
    cp_ax0 = pltpu.make_async_copy(ax_hbm.at[pl.ds(0, 256)], ax.at[pl.ds(0, 256)], sem_m.at[4])
    cp_ax1 = pltpu.make_async_copy(ax_hbm.at[pl.ds(256, _S - 256)], ax.at[pl.ds(256, _S - 256)],
                                   sem_m.at[5])
    cp_fd.start()
    cp_bx[0].start()
    cp_cm.start()
    for c in cp_bx[1:]:
        c.start()
    for c in cp_w:
        c.start()
    cp_fd.wait()
    cp_cm.wait()
    for c in cp_qkv:
        c.start()
    cp_ax0.start()
    for c in cp_wo:
        c.start()

    h2 = float(np.sqrt(0.5))

    def half(u, par):
        u = (u << 16) if par == 0 else (u & jnp.uint32(0xFFFF0000))
        return lax.bitcast_convert_type(u, F32)

    def forward(c, carry):
        pltpu.make_async_copy(bx_u32.at[:, c, :], bx.at[c], sem_m.at[6 + c]).wait()
        for par in range(2):
            a = 2 * c + par
            x = [half(bx[c, :, t * 128:(t + 1) * 128], par) for t in range(8)]
            e0, e1, e2, e3 = x[0] + x[4], x[0] - x[4], x[2] + x[6], x[2] - x[6]
            o0, o1, o2, o3 = x[1] + x[5], x[1] - x[5], x[3] + x[7], x[3] - x[7]
            ee, oo = e0 + e2, o0 + o2
            p, q = (o1 - o3) * h2, (o1 + o3) * h2
            ts = ((e1 + p, -(e3 + q)), (e0 - e2, o2 - o0), (e1 - p, e3 - q))
            re, im = [], []
            for g in range(3):
                t = jnp.concatenate([ts[g][0].astype(BF16), ts[g][1].astype(BF16)], axis=1)
                r = lax.dot_general(fd[g * 256:(g + 1) * 256, :], t, _NT,
                                    preferred_element_type=F32)
                re.append(r[0:128])
                im.append(r[128:256])
            r = lax.dot_general(fd[768:896, 0:128], (ee - oo).astype(BF16), _NT,
                                preferred_element_type=F32)
            re.append(r[0:64])
            im.append(r[64:128])
            r = lax.dot_general(fd[896:1040, 0:128], (ee + oo).astype(BF16), _NT,
                                preferred_element_type=F32)
            re.append(r[0:72])
            im.append(r[72:144])
            for r0, r1, g0, g1 in ((0, 256, 0, 2), (256, _KR, 2, 5)):
                u = jnp.concatenate([jnp.concatenate(re[g0:g1], axis=0),
                                     jnp.concatenate(im[g0:g1], axis=0)], axis=1)
                y[a, r0:r1, :] = jnp.dot(u, cm[a], preferred_element_type=F32)
        return carry

    lax.fori_loop(0, 8, forward, 0)
    for c in cp_w:
        c.wait()

    def spectral(rows, filt):
        xf = _dft16([(y[a, rows, 0:128], y[a, rows, 128:256]) for a in range(16)], -1)
        v = []
        for m1 in range(16):
            (xr, xi), (fr, fi) = xf[m1], filt(m1)
            v.append((xr * fr - xi * fi, xr * fi + xi * fr))
        res = _dft16(v, +1)
        for a in range(16):
            y[a, rows, 0:128] = res[a][0]
            y[a, rows, 128:256] = res[a][1]

    def spectral_pair(i, carry):
        c, jg = i // 8, i % 8
        w_rows = pl.ds(jg * 32 + c, 8, stride=4)
        for par in range(2):
            blk = _RES.index(par)
            for cc in range(1, 4):
                blk = jnp.where(c == cc, _RES.index(2 * cc + par), blk)
            spectral(pl.ds(pl.multiple_of(blk * 64 + jg * 8, 8), 8),
                     lambda m1: (half(wr[m1, w_rows, :], par), half(wi[m1, w_rows, :], par)))
        return carry

    lax.fori_loop(0, 32, spectral_pair, 0)
    spectral(pl.ds(512, 8),
             lambda m1: tuple(jnp.broadcast_to(w[0:1, m1 * 128:(m1 + 1) * 128].astype(F32), (8, 128))
                             for w in (wrn_ref, win_ref)))

    sign = jnp.where(lax.broadcasted_iota(jnp.int32, (128, 256), 0) % 2 == 0, 1.0, -1.0)

    def b_out_copy(c):
        return pltpu.make_async_copy(bx.at[c], out_u32.at[:, c, pl.ds(_D, _D)], sem_o.at[0])

    def inverse(c, carry):
        outs = []
        for par in range(2):
            a = 2 * c + par
            qs = []
            for g in range(3):
                z = lax.dot_general(cm[a], y[a, g * 128:(g + 1) * 128, :].astype(BF16), _NT,
                                    preferred_element_type=F32)
                r = jnp.dot(jnp.concatenate([z[0:128], z[128:256]], axis=1),
                            fd[g * 256:(g + 1) * 256, :], preferred_element_type=F32)
                qs.append((r[:, 0:128], r[:, 128:256]))
            (q1r, q1i), (q2r, q2i), (q3r, q3i) = qs
            z = lax.dot_general(cm[a], y[a, 384:512, :].astype(BF16), _NT,
                                preferred_element_type=F32)
            zr, zi = z[0:128], z[128:256]
            low = lax.broadcasted_iota(jnp.int32, (128, 128), 1) < 64
            r4 = jnp.dot(jnp.where(low, zr, pltpu.roll(zi, 64, 1)), fd[768:896, 0:128],
                         preferred_element_type=F32)
            r0 = jnp.dot(jnp.where(low, pltpu.roll(zr, 64, 1), zi), fd[768:896, 128:256],
                         preferred_element_type=F32)
            r0 = r0 + lax.dot_general(cm[a, 0:128, :], (y[a, 512:513, :] * sign).astype(BF16),
                                      _NT, preferred_element_type=F32)
            ee, oo = r0 + r4, r0 - r4
            e0, e2, o0, o2 = ee + q2r, ee - q2r, oo - q2i, oo + q2i
            e1, e3 = q1r + q3r, q3i - q1i
            p, q = (q1r - q3r) * h2, (q1i + q3i) * h2
            o1, o3 = p - q, -(p + q)
            cols = (e0 + e1, o0 + o1, e2 + e3, o2 + o3, e0 - e1, o0 - o1, e2 - e3, o2 - o3)
            outs.append([lax.bitcast_convert_type(v.astype(BF16).astype(F32), U32)
                         for v in cols])
        for t in range(8):
            bx[c, :, t * 128:(t + 1) * 128] = (outs[0][t] >> 16) | outs[1][t]
        return carry

    lax.fori_loop(0, 8, inverse, 0)

    for i in range(48):
        cp_qkv[i].wait()

        def repack(g, carry, i=i):
            src = pl.multiple_of(g * 128, 128)
            dst = pl.multiple_of(g * 64, 64)
            ev = wqkv[i + 1, pl.ds(src, 64, stride=2), :]
            od = wqkv[i + 1, pl.ds(src + 1, 64, stride=2), :]
            wqkv[i, pl.ds(dst, 64), :] = (ev & jnp.uint32(0xFFFF)) | (od << 16)
            wqkv[i, pl.ds(512 + dst, 64), :] = (ev >> 16) | (od & jnp.uint32(0xFFFF0000))
            return carry

        lax.fori_loop(0, 8, repack, 0, unroll=True)

    cp_ax0.wait()
    for c in cp_wo:
        c.wait()
    cp_ax1.start()
    for c in range(8):
        b_out_copy(c).start()

    qi = lax.broadcasted_iota(jnp.int32, (_L, _L), 0)
    ki = lax.broadcasted_iota(jnp.int32, (_L, _L), 1)
    mask = (qi < _M) | (qi >= ki)
    scale = 128 ** -0.5
    group, skew, lag = 8, 1, 2
    n_group = _H // group

    h_ref[0:_M, :] = mem_ref[...].astype(F32)
    h_ref[_M:_L, :] = ax[0:_SEG, :].astype(F32)

    def a_out_copy(s):
        rows = pl.ds(2 * s, 2)
        return pltpu.make_async_copy(ao.at[rows], out_hbm.at[rows, :, pl.ds(0, _D)],
                                     sem_o.at[1])

    def step(s, carry):
        @pl.when(s == 6)
        def _():
            cp_ax1.wait()

        st = {}

        def proj(j, hd):
            w = wqkv[j * 16 + hd // 2, (hd % 2) * 512:(hd % 2 + 1) * 512, :]
            st[j, hd] = jnp.dot(h_ref[...], pltpu.bitcast(w, BF16), preferred_element_type=F32)

        def scores(hd):
            sc = lax.dot_general(st[0, hd], st[1, hd], _NT, preferred_element_type=F32) * scale
            sc = jnp.where(mask, sc, -1000000000.0)
            p = jnp.exp(sc - jnp.max(sc, axis=1, keepdims=True))
            st['p', hd] = p
            st['l', hd] = 1.0 / jnp.sum(p, axis=1, keepdims=True)

        def pv(hd):
            o = jnp.dot(st['p', hd], st[2, hd], preferred_element_type=F32)
            ob_ref[:, hd * 128:(hd + 1) * 128] = o * st['l', hd]

        def w_out(g, n):
            lanes = slice(n * 128, (n + 1) * 128)
            w = wo[n, g * group * 64:(g + 1) * group * 64, :]
            r = jnp.dot(ob_ref[:, g * group * 128:(g + 1) * group * 128],
                        pltpu.bitcast(w, BF16), preferred_element_type=F32)
            if g > 0:
                r = r + acc_ref[:, lanes]
            if g < n_group - 1:
                acc_ref[:, lanes] = r
            else:
                h_ref[0:_M, lanes] = r[0:_M].astype(BF16).astype(F32)
                ao[2 * s, :, lanes] = r[_M:_M + 16].astype(BF16)
                ao[2 * s + 1, :, lanes] = r[_M + 16:_L].astype(BF16)

        def next_x():
            nxt = jnp.minimum(s + 1, _NSEG - 1)
            h_ref[_M:_L, :] = ax[pl.ds(pl.multiple_of(nxt * _SEG, _SEG), _SEG), :].astype(F32)

        ops, pending = [], []
        for t in range(_H + skew + lag):
            if t < _H:
                ops.append((proj, 0, t))
            if 1 <= t <= _H:
                ops.append((scores, t - 1))
            if t < _H:
                ops.append((proj, 1, t))
            if pending:
                ops.append(pending.pop(0))
            if 0 <= t - skew < _H:
                ops.append((proj, 2, t - skew))
            if t - skew == _H - 1:
                ops.append((next_x,))
            hd = t - skew - lag
            if hd == _H - 1:
                ops += pending
                pending = []
            if hd >= 0:
                ops.append((pv, hd))
                if hd % group == group - 1:
                    pending += [(w_out, hd // group, n) for n in range(8)]
        ops += pending
        for op in ops:
            op[0](*op[1:])
        a_out_copy(s).start()
        return carry

    lax.fori_loop(0, _NSEG, step, 0)

    def drain_b(a, carry):
        b_out_copy(a).wait()
        return carry

    def drain_a(s, carry):
        a_out_copy(s).wait()
        return carry

    lax.fori_loop(0, 8, drain_b, 0)
    lax.fori_loop(0, _NSEG, drain_a, 0)


@jax.jit
def _run(A_x, A_mem0, A_Wq, A_Wk, A_Wv, A_Wo, B_x, B_w_r, B_w_i):
    hbm = pl.BlockSpec(memory_space=pltpu.HBM)
    vmem = pl.BlockSpec(memory_space=pltpu.VMEM)
    nyquist = pl.BlockSpec((16, _S), lambda i: (512 // 16, 0))
    wr, wi = B_w_r.T, B_w_i.T
    out = pl.pallas_call(
        _kernel,
        grid=(1,),
        out_shape=jax.ShapeDtypeStruct((128, 16, 2 * _D), BF16),
        in_specs=[hbm, vmem, hbm, hbm, hbm, hbm, hbm, hbm, hbm, nyquist, nyquist, hbm, hbm],
        out_specs=hbm,
        scratch_shapes=[
            pltpu.VMEM((49, 1024, 128), U32),
            pltpu.VMEM((8, 2048, 128), U32),
            pltpu.VMEM((_S, _D), BF16),
            pltpu.VMEM((128, 16, _D), BF16),
            pltpu.VMEM((8, 128, _D), U32),
            pltpu.VMEM((16, 256, 128), U32),
            pltpu.VMEM((16, 256, 128), U32),
            pltpu.VMEM((1040, 256), BF16),
            pltpu.VMEM((16, 256, 256), BF16),
            pltpu.VMEM((16, _KR, 256), F32),
            pltpu.VMEM((_L, _D), F32),
            pltpu.VMEM((_L, _H * 128), F32),
            pltpu.VMEM((_L, _D), F32),
            pltpu.SemaphoreType.DMA((48,)),
            pltpu.SemaphoreType.DMA((14,)),
            pltpu.SemaphoreType.DMA((2,)),
        ],
        compiler_params=pltpu.CompilerParams(vmem_limit_bytes=100 * 1024 * 1024),
    )(A_x.reshape(_S, _D), A_mem0.reshape(_M, _D), A_Wq, A_Wk, A_Wv,
      A_Wo.reshape(_H * 128, _D), B_x.reshape(128, 16, _D), wr, wi, wr, wi, *_CONSTS)
    return out.reshape(1, _S, 2 * _D)


def pallas_concat_heads__memory_aug_recurrent_mem_tr__spectral_gfnet__prompt_kernel(
    A_x, A_mem0, A_Wq, A_Wk, A_Wv, A_Wo, A_seg_len, B_x, B_w_r, B_w_i,
):
    assert int(A_seg_len) == _SEG
    return _run(A_x, A_mem0, A_Wq, A_Wk, A_Wv, A_Wo, B_x, B_w_r, B_w_i)
```

```python
import numpy as np

import jax
import jax.numpy as jnp
from jax import lax
import jax.experimental.pallas as pl
import jax.experimental.pallas.tpu as pltpu

F32 = jnp.float32
BF16 = jnp.bfloat16
U32 = jnp.uint32

_S = 2048
_D = 1024
_H = 32
_M = 8
_SEG = 32
_L = _M + _SEG
_NSEG = _S // _SEG
_KR = 520
_RES = (1, 7, 2, 6, 3, 5, 4, 0)

_NT = (((1,), (1,)), ((), ()))


def _dft_constants():
    b = np.arange(128)

    def cs(k):
        ang = -2.0 * np.pi * ((k[:, None] * b[None, :]) % _D) / _D
        return np.cos(ang), np.sin(ang)

    j = np.arange(64)
    fd = np.zeros((1040, 256))
    for g, r in enumerate((1, 2, 3)):
        c1, s1 = cs(r + 8 * j)
        c2, s2 = cs(8 - r + 8 * j)
        fd[g * 256:(g + 1) * 256] = np.block([[c1, -s1], [c2, s2], [s1, c1], [s2, -c2]])
    c4, s4 = cs(4 + 8 * j)
    fd[768:896, :128] = np.concatenate([c4, s4], 0)
    c0, s0 = cs(8 * np.arange(72))
    c0[65:] = 0.0
    s0[64:] = 0.0
    s0[0] = 0.0
    fd[768:896, 128:] = np.concatenate([c0[:64], s0[:64]], 0)
    c0[0] *= 0.5
    c0[64] *= 0.5
    fd[896:1040, :128] = np.concatenate([c0, s0], 0)

    ang = -2.0 * np.pi * ((b[:, None] * b[None, :]) % 128) / 128
    tw = -2.0 * np.pi * ((np.arange(128) // 8)[:, None] * b[None, :]) / _S
    norm = np.sqrt(2.0 / (_S * _D))
    tab = np.block([[np.cos(ang), np.sin(ang)], [np.cos(tw) * norm, np.sin(tw) * norm]])
    return np.asarray(fd, np.float32).astype(BF16), np.asarray(tab, np.float32)


_CONSTS = _dft_constants()


def _dft4(x, sign):
    (ar, ai), (br, bi), (cr, ci), (dr, di) = x
    t0r, t0i, t1r, t1i = ar + cr, ai + ci, ar - cr, ai - ci
    t2r, t2i, t3r, t3i = br + dr, bi + di, br - dr, bi - di
    lo = (t1r + t3i, t1i - t3r)
    hi = (t1r - t3i, t1i + t3r)
    if sign > 0:
        lo, hi = hi, lo
    return [(t0r + t2r, t0i + t2i), lo, (t0r - t2r, t0i - t2i), hi]


def _twiddle16(z, e, sign):
    zr, zi = z
    if e == 0:
        return z
    if e == 4:
        return (-zi, zr) if sign > 0 else (zi, -zr)
    h = float(np.sqrt(0.5))
    if e == 2:
        return ((zr - zi) * h, (zr + zi) * h) if sign > 0 else ((zr + zi) * h, (zi - zr) * h)
    if e == 6:
        return ((zr + zi) * -h, (zr - zi) * h) if sign > 0 else ((zi - zr) * h, (zr + zi) * -h)
    c = float(np.cos(2 * np.pi * e / 16))
    s = float(sign * np.sin(2 * np.pi * e / 16))
    return (zr * c - zi * s, zr * s + zi * c)


def _dft16(x, sign):
    cols = [_dft4([x[n1 + 4 * n2] for n2 in range(4)], sign) for n1 in range(4)]
    out = [None] * 16
    for k2 in range(4):
        res = _dft4([_twiddle16(cols[n1][k2], n1 * k2, sign) for n1 in range(4)], sign)
        for k1 in range(4):
            out[k2 + 4 * k1] = res[k1]
    return out


def _kernel(ax_hbm, mem_ref, wq_hbm, wk_hbm, wv_hbm, wo_hbm, bx_hbm, wr_hbm, wi_hbm,
            wrn_ref, win_ref, fd_hbm, tab_ref, out_hbm,
            wqkv, wo, ax, ao, bx, wr, wi, fd, cm, y, xa, qa, h_ref, ob_ref, acc_ref,
            sem_w, sem_m, sem_o):
    qkv_u32 = [w.bitcast(U32) for w in (wq_hbm, wk_hbm, wv_hbm)]
    wo_u32 = wo_hbm.bitcast(U32)
    bx_u32 = bx_hbm.bitcast(U32)
    out_u32 = out_hbm.bitcast(U32)

    def bx_copy(c):
        return pltpu.make_async_copy(bx_u32.at[:, c, :], bx.at[c], sem_m.at[6 + c])

    def slab_copy(j, hp):
        return pltpu.make_async_copy(qkv_u32[j].at[:, hp, :], wqkv.at[j * 16 + hp + 1],
                                     sem_w.at[j * 16 + hp])

    def repair(i):
        for g in range(8):
            ev = wqkv[i + 1, pl.ds(g * 128, 64, stride=2), :]
            od = wqkv[i + 1, pl.ds(g * 128 + 1, 64, stride=2), :]
            wqkv[i, g * 64:(g + 1) * 64, :] = (ev & jnp.uint32(0xFFFF)) | (od << 16)
            wqkv[i, 512 + g * 64:512 + (g + 1) * 64, :] = (
                (ev >> 16) | (od & jnp.uint32(0xFFFF0000)))

    early = 8
    cp_fd = pltpu.make_async_copy(fd_hbm, fd, sem_m.at[0])

    def w_copies(c):
        return [pltpu.make_async_copy(
            src.at[pl.ds(0, 512)].bitcast(U32).at[:, pl.ds(pl.multiple_of(m1 * 128, 128), 128)],
            dst.at[m1], sem_m.at[2])
            for src, dst in ((wr_hbm, wr), (wi_hbm, wi)) for m1 in (2 * c, 2 * c + 1)]

    def wo_copy(n):
        return pltpu.make_async_copy(wo_u32.at[:, pl.ds(pl.multiple_of(n * 128, 128), 128)],
                                     wo.at[n], sem_m.at[3])

    cp_lo = pltpu.make_async_copy(ax_hbm.at[:, 0], ax.at[:, 0], sem_m.at[1])
    cp_hi0 = pltpu.make_async_copy(ax_hbm.at[pl.ds(0, early), 1], ax.at[pl.ds(0, early), 1],
                                   sem_m.at[4])
    cp_hi1 = pltpu.make_async_copy(ax_hbm.at[pl.ds(early, _NSEG - early), 1],
                                   ax.at[pl.ds(early, _NSEG - early), 1], sem_m.at[5])
    cp_fd.start()
    for c in range(3):
        bx_copy(c).start()

    h2 = float(np.sqrt(0.5))

    def half(u, par):
        u = (u << 16) if par == 0 else (u & jnp.uint32(0xFFFF0000))
        return lax.bitcast_convert_type(u, F32)

    def s_matrix(a, carry):
        c0, s0 = tab_ref[0:128, 0:128], tab_ref[0:128, 128:256]
        rows = pl.ds(pl.multiple_of(128 + 8 * a, 8), 8)
        tc, ts = tab_ref[rows, 0:128][0:1], tab_ref[rows, 128:256][0:1]
        cc, ss = c0 * tc - s0 * ts, c0 * ts + s0 * tc
        cm[a, 0:128, 0:128] = cc.astype(BF16)
        cm[a, 0:128, 128:256] = ss.astype(BF16)
        cm[a, 128:256, 0:128] = (-ss).astype(BF16)
        cm[a, 128:256, 128:256] = cc.astype(BF16)
        return carry

    lax.fori_loop(0, 16, s_matrix, 0)
    cp_fd.wait()

    def forward(c, carry):
        @pl.when(c < 5)
        def _():
            bx_copy(c + 3).start()

        @pl.when(c == 4)
        def _():
            cp_lo.start()

        @pl.when(c >= 5)
        def _():
            slab_copy(0, c - 5).start()

        for cp in w_copies(c):
            cp.start()
        bx_copy(c).wait()
        for par in range(2):
            a = 2 * c + par
            x = [half(bx[c, :, t * 128:(t + 1) * 128], par) for t in range(8)]
            e0, e1, e2, e3 = x[0] + x[4], x[0] - x[4], x[2] + x[6], x[2] - x[6]
            o0, o1, o2, o3 = x[1] + x[5], x[1] - x[5], x[3] + x[7], x[3] - x[7]
            ee, oo = e0 + e2, o0 + o2
            p, q = (o1 - o3) * h2, (o1 + o3) * h2
            ts = ((e1 + p, -(e3 + q)), (e0 - e2, o2 - o0), (e1 - p, e3 - q))
            re, im = [], []
            for g in range(3):
                t = jnp.concatenate([ts[g][0].astype(BF16), ts[g][1].astype(BF16)], axis=1)
                r = lax.dot_general(fd[g * 256:(g + 1) * 256, :], t, _NT,
                                    preferred_element_type=F32)
                re.append(r[0:128])
                im.append(r[128:256])
            r = lax.dot_general(fd[768:896, 0:128], (ee - oo).astype(BF16), _NT,
                                preferred_element_type=F32)
            re.append(r[0:64])
            im.append(r[64:128])
            r = lax.dot_general(fd[896:1040, 0:128], (ee + oo).astype(BF16), _NT,
                                preferred_element_type=F32)
            re.append(r[0:72])
            im.append(r[72:144])
            for r0, r1, g0, g1 in ((0, 256, 0, 2), (256, _KR, 2, 5)):
                u = jnp.concatenate([jnp.concatenate(re[g0:g1], axis=0),
                                     jnp.concatenate(im[g0:g1], axis=0)], axis=1)
                y[a, r0:r1, :] = jnp.dot(u, cm[a], preferred_element_type=F32)
        return carry

    lax.fori_loop(0, 8, forward, 0)
    slab_copy(0, 3).start()
    for c in range(8):
        for cp in w_copies(c):
            cp.wait()

    def spectral(rows, filt):
        xf = _dft16([(y[a, rows, 0:128], y[a, rows, 128:256]) for a in range(16)], -1)
        v = []
        for m1 in range(16):
            (xr, xi), (fr, fi) = xf[m1], filt(m1)
            v.append((xr * fr - xi * fi, xr * fi + xi * fr))
        res = _dft16(v, +1)
        for a in range(16):
            y[a, rows, 0:128] = res[a][0]
            y[a, rows, 128:256] = res[a][1]

    cp_lo.wait()
    for g in range(8):
        xa[g * 64:(g + 1) * 64, :] = (
            ax[g * 8:(g + 1) * 8, 0, :, :].astype(F32)[:, 0:8, :].reshape(64, _D).astype(BF16))
    slab_copy(0, 0).wait()
    repair(0)

    def middle(i, carry):
        @pl.when(i < 12)
        def _():
            slab_copy(0, i + 4).start()

        slab_copy(1, i).start()
        slab_copy(2, i).start()
        slab_copy(0, i + 1).wait()
        c = i // 4
        for par in range(2):
            w = pltpu.bitcast(wqkv[i, par * 512:(par + 1) * 512, :], BF16)
            qa[2 * i + par] = jnp.dot(xa[...], w, preferred_element_type=F32)
            blk = _RES.index(par)
            for cc in range(1, 4):
                blk = jnp.where(c == cc, _RES.index(2 * cc + par), blk)
            for jg in (2 * (i % 4), 2 * (i % 4) + 1):
                w_rows = pl.ds(jg * 32 + c, 8, stride=4)
                spectral(pl.ds(pl.multiple_of(blk * 64 + jg * 8, 8), 8),
                         lambda m1: (half(wr[m1, w_rows, :], par), half(wi[m1, w_rows, :], par)))
        repair(i + 1)
        return carry

    lax.fori_loop(0, 16, middle, 0)
    spectral(pl.ds(512, 8),
             lambda m1: tuple(jnp.broadcast_to(w[0:1, m1 * 128:(m1 + 1) * 128].astype(F32), (8, 128))
                             for w in (wrn_ref, win_ref)))

    sign = jnp.where(lax.broadcasted_iota(jnp.int32, (128, 256), 0) % 2 == 0, 1.0, -1.0)

    def b_out_copy(c):
        return pltpu.make_async_copy(bx.at[c], out_u32.at[:, c, pl.ds(_D, _D)], sem_o.at[0])

    def inverse(c, carry):
        wo_copy(c).start()
        slab_copy(0, 17 + 2 * c).wait()
        slab_copy(0, 18 + 2 * c).wait()
        zs = {}
        for par in range(2):
            a = 2 * c + par
            for g in range(4):
                z = lax.dot_general(cm[a], y[a, g * 128:(g + 1) * 128, :].astype(BF16), _NT,
                                    preferred_element_type=F32)
                zr, zi = z[0:128], z[128:256]
                if g < 3:
                    zs[par, g] = jnp.concatenate([zr, zi], axis=1).astype(BF16)
                else:
                    low = lax.broadcasted_iota(jnp.int32, (128, 128), 1) < 64
                    zs[par, 3] = jnp.where(low, zr, pltpu.roll(zi, 64, 1)).astype(BF16)
                    zs[par, 4] = jnp.where(low, pltpu.roll(zr, 64, 1), zi).astype(BF16)
            zs[par, 5] = lax.dot_general(
                cm[a, 0:128, :], (y[a, 512:513, :] * sign).astype(BF16), _NT,
                preferred_element_type=F32)
        outs = []
        for par in range(2):
            qs = []
            for g in range(3):
                r = jnp.dot(zs[par, g], fd[g * 256:(g + 1) * 256, :],
                            preferred_element_type=F32)
                qs.append((r[:, 0:128], r[:, 128:256]))
            (q1r, q1i), (q2r, q2i), (q3r, q3i) = qs
            r4 = jnp.dot(zs[par, 3], fd[768:896, 0:128], preferred_element_type=F32)
            r0 = jnp.dot(zs[par, 4], fd[768:896, 128:256],
                         preferred_element_type=F32) + zs[par, 5]
            ee, oo = r0 + r4, r0 - r4
            e0, e2, o0, o2 = ee + q2r, ee - q2r, oo - q2i, oo + q2i
            e1, e3 = q1r + q3r, q3i - q1i
            p, q = (q1r - q3r) * h2, (q1i + q3i) * h2
            o1, o3 = p - q, -(p + q)
            cols = (e0 + e1, o0 + o1, e2 + e3, o2 + o3, e0 - e1, o0 - o1, e2 - e3, o2 - o3)
            outs.append([lax.bitcast_convert_type(v.astype(BF16).astype(F32), U32)
                         for v in cols])
        for t in range(8):
            bx[c, :, t * 128:(t + 1) * 128] = (outs[0][t] >> 16) | outs[1][t]
        repair(17 + 2 * c)
        repair(18 + 2 * c)
        return carry

    cp_hi0.start()
    lax.fori_loop(0, 8, inverse, 0)

    def last_slabs(i, carry):
        slab_copy(0, i).wait()
        repair(i)
        return carry

    lax.fori_loop(33, 48, last_slabs, 0)
    cp_hi0.wait()
    for n in range(8):
        wo_copy(n).wait()
    cp_hi1.start()
    for c in range(8):
        b_out_copy(c).start()

    def position(i):
        return jnp.where(i < 8, i + _M, jnp.where(i < 8 + _M, i - 8, i))

    qi = position(lax.broadcasted_iota(jnp.int32, (_L, _L), 0))
    ki = position(lax.broadcasted_iota(jnp.int32, (_L, _L), 1))
    mask = (qi < _M) | (qi >= ki)
    scale = 128 ** -0.5
    group, skew, lag = 8, 1, 2
    n_group = _H // group

    def load_tokens(s):
        lo = ax[s, 0].astype(F32)
        h_ref[0:8, :] = lo[0:8]
        h_ref[16:24, :] = lo[8:16]
        h_ref[24:40, :] = ax[s, 1].astype(F32)

    h_ref[8:16, :] = mem_ref[...].astype(F32)
    load_tokens(0)

    def a_out_copy(s):
        rows = pl.ds(2 * s, 2)
        return pltpu.make_async_copy(ao.at[rows], out_hbm.at[rows, :, pl.ds(0, _D)],
                                     sem_o.at[1])

    def step(s, carry):
        @pl.when(s == early - 1)
        def _():
            cp_hi1.wait()

        st = {}

        def proj(j, hd):
            w = wqkv[j * 16 + hd // 2, (hd % 2) * 512:(hd % 2 + 1) * 512, :]
            r = jnp.dot(h_ref[(8 if j == 0 else 0):_L, :], pltpu.bitcast(w, BF16),
                        preferred_element_type=F32)
            if j == 0:
                r = jnp.concatenate([qa[hd, pl.ds(pl.multiple_of(s * 8, 8), 8), :], r], axis=0)
            st[j, hd] = r

        def scores(hd):
            sc = lax.dot_general(st[0, hd], st[1, hd], _NT, preferred_element_type=F32) * scale
            sc = jnp.where(mask, sc, -1000000000.0)
            p = jnp.exp(sc - jnp.max(sc, axis=1, keepdims=True))
            st['p', hd] = p
            st['l', hd] = 1.0 / jnp.sum(p, axis=1, keepdims=True)

        def pv(hd):
            o = jnp.dot(st['p', hd], st[2, hd], preferred_element_type=F32)
            ob_ref[:, hd * 128:(hd + 1) * 128] = o * st['l', hd]

        def w_out(g, n):
            lanes = slice(n * 128, (n + 1) * 128)
            w = wo[n, g * group * 64:(g + 1) * group * 64, :]
            r = jnp.dot(ob_ref[:, g * group * 128:(g + 1) * group * 128],
                        pltpu.bitcast(w, BF16), preferred_element_type=F32)
            if g > 0:
                r = r + acc_ref[:, lanes]
            if g < n_group - 1:
                acc_ref[:, lanes] = r
            else:
                h_ref[8:16, lanes] = r[8:16].astype(BF16).astype(F32)
                ao[2 * s, :, lanes] = jnp.concatenate([r[0:8], r[16:24]], axis=0).astype(BF16)
                ao[2 * s + 1, :, lanes] = r[24:40].astype(BF16)

        def next_x():
            load_tokens(jnp.minimum(s + 1, _NSEG - 1))

        ops, pending = [], []
        for t in range(_H + skew + lag):
            if t < _H:
                ops.append((proj, 0, t))
            if 1 <= t <= _H:
                ops.append((scores, t - 1))
            if t < _H:
                ops.append((proj, 1, t))
            if pending:
                ops.append(pending.pop(0))
            if 0 <= t - skew < _H:
                ops.append((proj, 2, t - skew))
            if t - skew == _H - 1:
                ops.append((next_x,))
            hd = t - skew - lag
            if hd == _H - 1:
                ops += pending
                pending = []
            if hd >= 0:
                ops.append((pv, hd))
                if hd % group == group - 1:
                    pending += [(w_out, hd // group, n) for n in range(8)]
        ops += pending
        for op in ops:
            op[0](*op[1:])
        a_out_copy(s).start()
        return carry

    lax.fori_loop(0, _NSEG, step, 0)

    def drain_b(a, carry):
        b_out_copy(a).wait()
        return carry

    def drain_a(s, carry):
        a_out_copy(s).wait()
        return carry

    lax.fori_loop(0, 8, drain_b, 0)
    lax.fori_loop(0, _NSEG, drain_a, 0)


@jax.jit
def _run(A_x, A_mem0, A_Wq, A_Wk, A_Wv, A_Wo, B_x, B_w_r, B_w_i):
    hbm = pl.BlockSpec(memory_space=pltpu.HBM)
    vmem = pl.BlockSpec(memory_space=pltpu.VMEM)
    nyquist = pl.BlockSpec((16, _S), lambda i: (512 // 16, 0))
    wr, wi = B_w_r.T, B_w_i.T
    out = pl.pallas_call(
        _kernel,
        grid=(1,),
        out_shape=jax.ShapeDtypeStruct((128, 16, 2 * _D), BF16),
        in_specs=[hbm, vmem, hbm, hbm, hbm, hbm, hbm, hbm, hbm, nyquist, nyquist, hbm, vmem],
        out_specs=hbm,
        scratch_shapes=[
            pltpu.VMEM((49, 1024, 128), U32),
            pltpu.VMEM((8, 2048, 128), U32),
            pltpu.VMEM((_NSEG, 2, 16, _D), BF16),
            pltpu.VMEM((128, 16, _D), BF16),
            pltpu.VMEM((8, 128, _D), U32),
            pltpu.VMEM((16, 256, 128), U32),
            pltpu.VMEM((16, 256, 128), U32),
            pltpu.VMEM((1040, 256), BF16),
            pltpu.VMEM((16, 256, 256), BF16),
            pltpu.VMEM((16, _KR, 256), F32),
            pltpu.VMEM((_NSEG * 8, _D), BF16),
            pltpu.VMEM((_H, _NSEG * 8, 128), F32),
            pltpu.VMEM((_L, _D), F32),
            pltpu.VMEM((_L, _H * 128), F32),
            pltpu.VMEM((_L, _D), F32),
            pltpu.SemaphoreType.DMA((48,)),
            pltpu.SemaphoreType.DMA((14,)),
            pltpu.SemaphoreType.DMA((2,)),
        ],
        compiler_params=pltpu.CompilerParams(vmem_limit_bytes=100 * 1024 * 1024),
    )(A_x.reshape(_NSEG, 2, 16, _D), A_mem0.reshape(_M, _D), A_Wq, A_Wk, A_Wv,
      A_Wo.reshape(_H * 128, _D), B_x.reshape(128, 16, _D), wr, wi, wr, wi, *_CONSTS)
    return out.reshape(1, _S, 2 * _D)


def pallas_concat_heads__memory_aug_recurrent_mem_tr__spectral_gfnet__prompt_kernel(
    A_x, A_mem0, A_Wq, A_Wk, A_Wv, A_Wo, A_seg_len, B_x, B_w_r, B_w_i,
):
    assert int(A_seg_len) == _SEG
    return _run(A_x, A_mem0, A_Wq, A_Wk, A_Wv, A_Wo, B_x, B_w_r, B_w_i)
```

```python
import numpy as np

import jax
import jax.numpy as jnp
from jax import lax
import jax.experimental.pallas as pl
import jax.experimental.pallas.tpu as pltpu

F32 = jnp.float32
BF16 = jnp.bfloat16
U32 = jnp.uint32

_S = 2048
_D = 1024
_H = 32
_M = 8
_SEG = 32
_L = _M + _SEG
_NSEG = _S // _SEG
_KR = 520
_RES = (1, 7, 2, 6, 3, 5, 4, 0)

_NT = (((1,), (1,)), ((), ()))


def _dft_constants():
    b = np.arange(128)

    def cs(k):
        ang = -2.0 * np.pi * ((k[:, None] * b[None, :]) % _D) / _D
        return np.cos(ang), np.sin(ang)

    j = np.arange(64)
    fd = np.zeros((1040, 256))
    for g, r in enumerate((1, 2, 3)):
        c1, s1 = cs(r + 8 * j)
        c2, s2 = cs(8 - r + 8 * j)
        fd[g * 256:(g + 1) * 256] = np.block([[c1, -s1], [c2, s2], [s1, c1], [s2, -c2]])
    c4, s4 = cs(4 + 8 * j)
    fd[768:896, :128] = np.concatenate([c4, s4], 0)
    c0, s0 = cs(8 * np.arange(72))
    c0[65:] = 0.0
    s0[64:] = 0.0
    s0[0] = 0.0
    fd[768:896, 128:] = np.concatenate([c0[:64], s0[:64]], 0)
    c0[0] *= 0.5
    c0[64] *= 0.5
    fd[896:1040, :128] = np.concatenate([c0, s0], 0)

    ang = -2.0 * np.pi * ((b[:, None] * b[None, :]) % 128) / 128
    tw = -2.0 * np.pi * ((np.arange(128) // 8)[:, None] * b[None, :]) / _S
    norm = np.sqrt(2.0 / (_S * _D))
    tab = np.block([[np.cos(ang), np.sin(ang)], [np.cos(tw) * norm, np.sin(tw) * norm]])
    return np.asarray(fd, np.float32).astype(BF16), np.asarray(tab, np.float32)


_CONSTS = _dft_constants()


def _dft4(x, sign):
    (ar, ai), (br, bi), (cr, ci), (dr, di) = x
    t0r, t0i, t1r, t1i = ar + cr, ai + ci, ar - cr, ai - ci
    t2r, t2i, t3r, t3i = br + dr, bi + di, br - dr, bi - di
    lo = (t1r + t3i, t1i - t3r)
    hi = (t1r - t3i, t1i + t3r)
    if sign > 0:
        lo, hi = hi, lo
    return [(t0r + t2r, t0i + t2i), lo, (t0r - t2r, t0i - t2i), hi]


def _twiddle16(z, e, sign):
    zr, zi = z
    if e == 0:
        return z
    if e == 4:
        return (-zi, zr) if sign > 0 else (zi, -zr)
    h = float(np.sqrt(0.5))
    if e == 2:
        return ((zr - zi) * h, (zr + zi) * h) if sign > 0 else ((zr + zi) * h, (zi - zr) * h)
    if e == 6:
        return ((zr + zi) * -h, (zr - zi) * h) if sign > 0 else ((zi - zr) * h, (zr + zi) * -h)
    c = float(np.cos(2 * np.pi * e / 16))
    s = float(sign * np.sin(2 * np.pi * e / 16))
    return (zr * c - zi * s, zr * s + zi * c)


def _dft16(x, sign):
    cols = [_dft4([x[n1 + 4 * n2] for n2 in range(4)], sign) for n1 in range(4)]
    out = [None] * 16
    for k2 in range(4):
        res = _dft4([_twiddle16(cols[n1][k2], n1 * k2, sign) for n1 in range(4)], sign)
        for k1 in range(4):
            out[k2 + 4 * k1] = res[k1]
    return out


def _kernel(ax_hbm, mem_ref, wq_hbm, wk_hbm, wv_hbm, wo_hbm, bx_hbm, wr_hbm, wi_hbm,
            wrn_ref, win_ref, fd_hbm, tab_ref, out_hbm,
            wqkv, wo, ax, ao, bx, wr, wi, fd, cm, y, xa, qa, h_ref, ob_ref, acc_ref,
            sem_w, sem_m, sem_o):
    qkv_u32 = [w.bitcast(U32) for w in (wq_hbm, wk_hbm, wv_hbm)]
    wo_u32 = wo_hbm.bitcast(U32)
    bx_u32 = bx_hbm.bitcast(U32)
    out_u32 = out_hbm.bitcast(U32)

    def bx_copy(c):
        return pltpu.make_async_copy(bx_u32.at[:, c, :], bx.at[c], sem_m.at[6 + c])

    def slab_copy(j, hp):
        return pltpu.make_async_copy(qkv_u32[j].at[:, hp, :], wqkv.at[j * 16 + hp + 1],
                                     sem_w.at[j * 16 + hp])

    def repair(i):
        for g in range(8):
            ev = wqkv[i + 1, pl.ds(g * 128, 64, stride=2), :]
            od = wqkv[i + 1, pl.ds(g * 128 + 1, 64, stride=2), :]
            wqkv[i, g * 64:(g + 1) * 64, :] = (ev & jnp.uint32(0xFFFF)) | (od << 16)
            wqkv[i, 512 + g * 64:512 + (g + 1) * 64, :] = (
                (ev >> 16) | (od & jnp.uint32(0xFFFF0000)))

    early = 8
    cp_fd = pltpu.make_async_copy(fd_hbm, fd, sem_m.at[0])

    def w_copies(c):
        return [pltpu.make_async_copy(
            src.at[pl.ds(0, 512)].bitcast(U32).at[:, pl.ds(pl.multiple_of(m1 * 128, 128), 128)],
            dst.at[m1], sem_m.at[2])
            for src, dst in ((wr_hbm, wr), (wi_hbm, wi)) for m1 in (2 * c, 2 * c + 1)]

    def wo_copy(n):
        return pltpu.make_async_copy(wo_u32.at[:, pl.ds(pl.multiple_of(n * 128, 128), 128)],
                                     wo.at[n], sem_m.at[3])

    cp_lo = pltpu.make_async_copy(ax_hbm.at[:, 0], ax.at[:, 0], sem_m.at[1])
    cp_hi0, cp_hi1 = (
        pltpu.make_async_copy(ax_hbm.at[segs, pl.ds(1, 3)], ax.at[segs, pl.ds(1, 3)], sem_m.at[k])
        for segs, k in ((pl.ds(0, early), 4), (pl.ds(early, _NSEG - early), 5)))
    cp_fd.start()
    for c in range(3):
        bx_copy(c).start()
    for cp in w_copies(0):
        cp.start()

    h2 = float(np.sqrt(0.5))

    def half(u, par):
        u = (u << 16) if par == 0 else (u & jnp.uint32(0xFFFF0000))
        return lax.bitcast_convert_type(u, F32)

    def s_matrix(a, carry):
        c0, s0 = tab_ref[0:128, 0:128], tab_ref[0:128, 128:256]
        rows = pl.ds(pl.multiple_of(128 + 8 * a, 8), 8)
        tc, ts = tab_ref[rows, 0:128][0:1], tab_ref[rows, 128:256][0:1]
        cc, ss = c0 * tc - s0 * ts, c0 * ts + s0 * tc
        cm[a, 0:128, 0:128] = cc.astype(BF16)
        cm[a, 0:128, 128:256] = ss.astype(BF16)
        cm[a, 128:256, 0:128] = (-ss).astype(BF16)
        cm[a, 128:256, 128:256] = cc.astype(BF16)
        return carry

    lax.fori_loop(0, 16, s_matrix, 0)
    cp_fd.wait()

    def forward(c, carry):
        @pl.when(c < 5)
        def _():
            bx_copy(c + 3).start()

        @pl.when(c < 7)
        def _():
            for cp in w_copies(c + 1):
                cp.start()

        @pl.when(c >= 5)
        def _():
            slab_copy(0, c - 5).start()

        @pl.when(c == 5)
        def _():
            cp_lo.start()

        bx_copy(c).wait()
        for par in range(2):
            a = 2 * c + par
            x = [half(bx[c, :, t * 128:(t + 1) * 128], par) for t in range(8)]
            e0, e1, e2, e3 = x[0] + x[4], x[0] - x[4], x[2] + x[6], x[2] - x[6]
            o0, o1, o2, o3 = x[1] + x[5], x[1] - x[5], x[3] + x[7], x[3] - x[7]
            ee, oo = e0 + e2, o0 + o2
            p, q = (o1 - o3) * h2, (o1 + o3) * h2
            ts = ((e1 + p, -(e3 + q)), (e0 - e2, o2 - o0), (e1 - p, e3 - q))
            re, im = [], []
            for g in range(3):
                t = jnp.concatenate([ts[g][0].astype(BF16), ts[g][1].astype(BF16)], axis=1)
                r = lax.dot_general(fd[g * 256:(g + 1) * 256, :], t, _NT,
                                    preferred_element_type=F32)
                re.append(r[0:128])
                im.append(r[128:256])
            r = lax.dot_general(fd[768:896, 0:128], (ee - oo).astype(BF16), _NT,
                                preferred_element_type=F32)
            re.append(r[0:64])
            im.append(r[64:128])
            r = lax.dot_general(fd[896:1040, 0:128], (ee + oo).astype(BF16), _NT,
                                preferred_element_type=F32)
            re.append(r[0:72])
            im.append(r[72:144])
            for r0, r1, g0, g1 in ((0, 256, 0, 2), (256, _KR, 2, 5)):
                u = jnp.concatenate([jnp.concatenate(re[g0:g1], axis=0),
                                     jnp.concatenate(im[g0:g1], axis=0)], axis=1)
                y[a, r0:r1, :] = jnp.dot(u, cm[a], preferred_element_type=F32)
        return carry

    lax.fori_loop(0, 8, forward, 0)
    slab_copy(0, 3).start()
    for c in range(8):
        for cp in w_copies(c):
            cp.wait()

    def spectral(rows, filt):
        xf = _dft16([(y[a, rows, 0:128], y[a, rows, 128:256]) for a in range(16)], -1)
        v = []
        for m1 in range(16):
            (xr, xi), (fr, fi) = xf[m1], filt(m1)
            v.append((xr * fr - xi * fi, xr * fi + xi * fr))
        res = _dft16(v, +1)
        for a in range(16):
            y[a, rows, 0:128] = res[a][0]
            y[a, rows, 128:256] = res[a][1]

    cp_lo.wait()
    for g in range(8):
        xa[g * 64:(g + 1) * 64, :] = (
            ax[g * 8:(g + 1) * 8, 0, :, :].astype(F32).reshape(64, _D).astype(BF16))
    slab_copy(0, 0).wait()
    repair(0)

    def middle(i, carry):
        @pl.when(i < 12)
        def _():
            slab_copy(0, i + 4).start()

        slab_copy(1, i).start()
        slab_copy(2, i).start()
        slab_copy(0, i + 1).wait()
        c = i // 4
        for par in range(2):
            w = pltpu.bitcast(wqkv[i, par * 512:(par + 1) * 512, :], BF16)
            qa[2 * i + par] = jnp.dot(xa[...], w, preferred_element_type=F32)
            blk = _RES.index(par)
            for cc in range(1, 4):
                blk = jnp.where(c == cc, _RES.index(2 * cc + par), blk)
            for jg in (2 * (i % 4), 2 * (i % 4) + 1):
                w_rows = pl.ds(jg * 32 + c, 8, stride=4)
                spectral(pl.ds(pl.multiple_of(blk * 64 + jg * 8, 8), 8),
                         lambda m1: (half(wr[m1, w_rows, :], par), half(wi[m1, w_rows, :], par)))
        repair(i + 1)
        return carry

    lax.fori_loop(0, 16, middle, 0)
    spectral(pl.ds(512, 8),
             lambda m1: tuple(jnp.broadcast_to(w[0:1, m1 * 128:(m1 + 1) * 128].astype(F32), (8, 128))
                             for w in (wrn_ref, win_ref)))

    sign = jnp.where(lax.broadcasted_iota(jnp.int32, (128, 256), 0) % 2 == 0, 1.0, -1.0)

    def b_out_copy(c):
        return pltpu.make_async_copy(bx.at[c], out_u32.at[:, c, pl.ds(_D, _D)], sem_o.at[0])

    def inverse(c, carry):
        wo_copy(c).start()
        slab_copy(0, 17 + 2 * c).wait()
        slab_copy(0, 18 + 2 * c).wait()
        zs = {}
        for par in range(2):
            a = 2 * c + par
            for g in range(4):
                z = lax.dot_general(cm[a], y[a, g * 128:(g + 1) * 128, :].astype(BF16), _NT,
                                    preferred_element_type=F32)
                zr, zi = z[0:128], z[128:256]
                if g < 3:
                    zs[par, g] = jnp.concatenate([zr, zi], axis=1).astype(BF16)
                else:
                    low = lax.broadcasted_iota(jnp.int32, (128, 128), 1) < 64
                    zs[par, 3] = jnp.where(low, zr, pltpu.roll(zi, 64, 1)).astype(BF16)
                    zs[par, 4] = jnp.where(low, pltpu.roll(zr, 64, 1), zi).astype(BF16)
            zs[par, 5] = lax.dot_general(
                cm[a, 0:128, :], (y[a, 512:513, :] * sign).astype(BF16), _NT,
                preferred_element_type=F32)
        outs = []
        for par in range(2):
            qs = []
            for g in range(3):
                r = jnp.dot(zs[par, g], fd[g * 256:(g + 1) * 256, :],
                            preferred_element_type=F32)
                qs.append((r[:, 0:128], r[:, 128:256]))
            (q1r, q1i), (q2r, q2i), (q3r, q3i) = qs
            r4 = jnp.dot(zs[par, 3], fd[768:896, 0:128], preferred_element_type=F32)
            r0 = jnp.dot(zs[par, 4], fd[768:896, 128:256],
                         preferred_element_type=F32) + zs[par, 5]
            ee, oo = r0 + r4, r0 - r4
            e0, e2, o0, o2 = ee + q2r, ee - q2r, oo - q2i, oo + q2i
            e1, e3 = q1r + q3r, q3i - q1i
            p, q = (q1r - q3r) * h2, (q1i + q3i) * h2
            o1, o3 = p - q, -(p + q)
            cols = (e0 + e1, o0 + o1, e2 + e3, o2 + o3, e0 - e1, o0 - o1, e2 - e3, o2 - o3)
            outs.append([lax.bitcast_convert_type(v.astype(BF16).astype(F32), U32)
                         for v in cols])
        for t in range(8):
            bx[c, :, t * 128:(t + 1) * 128] = (outs[0][t] >> 16) | outs[1][t]
        repair(17 + 2 * c)
        repair(18 + 2 * c)
        return carry

    cp_hi0.start()
    lax.fori_loop(0, 8, inverse, 0)

    def last_slabs(i, carry):
        slab_copy(0, i).wait()
        repair(i)
        return carry

    lax.fori_loop(33, 48, last_slabs, 0)
    cp_hi0.wait()
    for n in range(8):
        wo_copy(n).wait()
    cp_hi1.start()
    for c in range(8):
        b_out_copy(c).start()

    def position(i):
        return jnp.where(i < 8, i + _M, jnp.where(i < 8 + _M, i - 8, i))

    qi = position(lax.broadcasted_iota(jnp.int32, (_L, _L), 0))
    ki = position(lax.broadcasted_iota(jnp.int32, (_L, _L), 1))
    mask = (qi < _M) | (qi >= ki)
    scale = 128 ** -0.5
    group, skew, lag, slag, order = 8, 1, 2, 1, 'kqsvop'
    n_group = _H // group

    def load_tokens(s):
        for k, r0 in enumerate((0, 16, 24, 32)):
            h_ref[r0:r0 + 8, :] = ax[s, k].astype(F32)

    h_ref[8:16, :] = mem_ref[...].astype(F32)
    load_tokens(0)

    def a_out_copy(s):
        rows = pl.ds(2 * s, 2)
        return pltpu.make_async_copy(ao.at[rows], out_hbm.at[rows, :, pl.ds(0, _D)],
                                     sem_o.at[1])

    def step(s, carry):
        @pl.when(s == early - 1)
        def _():
            cp_hi1.wait()

        st = {}

        def proj(j, hd):
            w = wqkv[j * 16 + hd // 2, (hd % 2) * 512:(hd % 2 + 1) * 512, :]
            r = jnp.dot(h_ref[(8 if j == 0 else 0):_L, :], pltpu.bitcast(w, BF16),
                        preferred_element_type=F32)
            if j == 0:
                r = jnp.concatenate([qa[hd, pl.ds(pl.multiple_of(s * 8, 8), 8), :], r], axis=0)
            st[j, hd] = r

        def scores(hd):
            sc = lax.dot_general(st[0, hd], st[1, hd], _NT, preferred_element_type=F32) * scale
            sc = jnp.where(mask, sc, -1000000000.0)
            p = jnp.exp(sc - jnp.max(sc, axis=1, keepdims=True))
            st['p', hd] = p
            st['l', hd] = 1.0 / jnp.sum(p, axis=1, keepdims=True)

        def pv(hd):
            o = jnp.dot(st['p', hd], st[2, hd], preferred_element_type=F32)
            ob_ref[:, hd * 128:(hd + 1) * 128] = o * st['l', hd]

        def w_out(g, n):
            lanes = slice(n * 128, (n + 1) * 128)
            w = wo[n, g * group * 64:(g + 1) * group * 64, :]
            r = jnp.dot(ob_ref[:, g * group * 128:(g + 1) * group * 128],
                        pltpu.bitcast(w, BF16), preferred_element_type=F32)
            if g > 0:
                r = r + acc_ref[:, lanes]
            if g < n_group - 1:
                acc_ref[:, lanes] = r
            else:
                h_ref[8:16, lanes] = r[8:16].astype(BF16).astype(F32)
                ao[2 * s, :, lanes] = jnp.concatenate([r[0:8], r[16:24]], axis=0).astype(BF16)
                ao[2 * s + 1, :, lanes] = r[24:40].astype(BF16)

        def next_x():
            load_tokens(jnp.minimum(s + 1, _NSEG - 1))

        ops, pending = [], []
        for t in range(_H + skew + lag + slag):
            for what in order:
                if what == 'q' and t < _H:
                    ops.append((proj, 0, t))
                if what == 'k' and t < _H:
                    ops.append((proj, 1, t))
                if what == 's' and 0 <= t - slag < _H:
                    ops.append((scores, t - slag))
                if what == 'o' and pending:
                    ops.append(pending.pop(0))
                if what == 'v' and 0 <= t - skew < _H:
                    ops.append((proj, 2, t - skew))
                    if t - skew == _H - 1:
                        ops.append((next_x,))
                hd = t - skew - lag
                if what == 'p' and 0 <= hd < _H:
                    if hd == _H - 1:
                        ops += pending
                        pending = []
                    ops.append((pv, hd))
                    if hd % group == group - 1:
                        pending += [(w_out, hd // group, n) for n in range(8)]
        ops += pending
        for op in ops:
            op[0](*op[1:])
        a_out_copy(s).start()
        return carry

    lax.fori_loop(0, _NSEG, step, 0)

    def drain_b(a, carry):
        b_out_copy(a).wait()
        return carry

    def drain_a(s, carry):
        a_out_copy(s).wait()
        return carry

    lax.fori_loop(0, 8, drain_b, 0)
    lax.fori_loop(0, _NSEG, drain_a, 0)


@jax.jit
def _run(A_x, A_mem0, A_Wq, A_Wk, A_Wv, A_Wo, B_x, B_w_r, B_w_i):
    hbm = pl.BlockSpec(memory_space=pltpu.HBM)
    vmem = pl.BlockSpec(memory_space=pltpu.VMEM)
    nyquist = pl.BlockSpec((16, _S), lambda i: (512 // 16, 0))
    wr, wi = B_w_r.T, B_w_i.T
    out = pl.pallas_call(
        _kernel,
        grid=(1,),
        out_shape=jax.ShapeDtypeStruct((128, 16, 2 * _D), BF16),
        in_specs=[hbm, vmem, hbm, hbm, hbm, hbm, hbm, hbm, hbm, nyquist, nyquist, hbm, vmem],
        out_specs=hbm,
        scratch_shapes=[
            pltpu.VMEM((49, 1024, 128), U32),
            pltpu.VMEM((8, 2048, 128), U32),
            pltpu.VMEM((_NSEG, 4, 8, _D), BF16),
            pltpu.VMEM((128, 16, _D), BF16),
            pltpu.VMEM((8, 128, _D), U32),
            pltpu.VMEM((16, 256, 128), U32),
            pltpu.VMEM((16, 256, 128), U32),
            pltpu.VMEM((1040, 256), BF16),
            pltpu.VMEM((16, 256, 256), BF16),
            pltpu.VMEM((16, _KR, 256), F32),
            pltpu.VMEM((_NSEG * 8, _D), BF16),
            pltpu.VMEM((_H, _NSEG * 8, 128), F32),
            pltpu.VMEM((_L, _D), F32),
            pltpu.VMEM((_L, _H * 128), F32),
            pltpu.VMEM((_L, _D), F32),
            pltpu.SemaphoreType.DMA((48,)),
            pltpu.SemaphoreType.DMA((14,)),
            pltpu.SemaphoreType.DMA((2,)),
        ],
        compiler_params=pltpu.CompilerParams(vmem_limit_bytes=100 * 1024 * 1024),
    )(A_x.reshape(_NSEG, 4, 8, _D), A_mem0.reshape(_M, _D), A_Wq, A_Wk, A_Wv,
      A_Wo.reshape(_H * 128, _D), B_x.reshape(128, 16, _D), wr, wi, wr, wi, *_CONSTS)
    return out.reshape(1, _S, 2 * _D)


def pallas_concat_heads__memory_aug_recurrent_mem_tr__spectral_gfnet__prompt_kernel(
    A_x, A_mem0, A_Wq, A_Wk, A_Wv, A_Wo, A_seg_len, B_x, B_w_r, B_w_i,
):
    assert int(A_seg_len) == _SEG
    return _run(A_x, A_mem0, A_Wq, A_Wk, A_Wv, A_Wo, B_x, B_w_r, B_w_i)
```

```python
import numpy as np

import jax
import jax.numpy as jnp
from jax import lax
import jax.experimental.pallas as pl
import jax.experimental.pallas.tpu as pltpu

F32 = jnp.float32
BF16 = jnp.bfloat16
U32 = jnp.uint32

_S = 2048
_D = 1024
_H = 32
_M = 8
_SEG = 32
_L = _M + _SEG
_NSEG = _S // _SEG
_KR = 520
_RES = (1, 7, 2, 6, 3, 5, 4, 0)

_NT = (((1,), (1,)), ((), ()))


def _dft_constants():
    b = np.arange(128)

    def cs(k):
        ang = -2.0 * np.pi * ((k[:, None] * b[None, :]) % _D) / _D
        return np.cos(ang), np.sin(ang)

    j = np.arange(64)
    fd = np.zeros((1040, 256))
    for g, r in enumerate((1, 2, 3)):
        c1, s1 = cs(r + 8 * j)
        c2, s2 = cs(8 - r + 8 * j)
        fd[g * 256:(g + 1) * 256] = np.block([[c1, -s1], [c2, s2], [s1, c1], [s2, -c2]])
    c4, s4 = cs(4 + 8 * j)
    fd[768:896, :128] = np.concatenate([c4, s4], 0)
    c0, s0 = cs(8 * np.arange(72))
    c0[65:] = 0.0
    s0[64:] = 0.0
    s0[0] = 0.0
    fd[768:896, 128:] = np.concatenate([c0[:64], s0[:64]], 0)
    c0[0] *= 0.5
    c0[64] *= 0.5
    fd[896:1040, :128] = np.concatenate([c0, s0], 0)

    ang = -2.0 * np.pi * ((b[:, None] * b[None, :]) % 128) / 128
    tw = -2.0 * np.pi * ((np.arange(128) // 8)[:, None] * b[None, :]) / _S
    norm = np.sqrt(2.0 / (_S * _D))
    tab = np.block([[np.cos(ang), np.sin(ang)], [np.cos(tw) * norm, np.sin(tw) * norm]])
    return np.asarray(fd, np.float32).astype(BF16), np.asarray(tab, np.float32)


_CONSTS = _dft_constants()


def _dft4(x, sign):
    (ar, ai), (br, bi), (cr, ci), (dr, di) = x
    t0r, t0i, t1r, t1i = ar + cr, ai + ci, ar - cr, ai - ci
    t2r, t2i, t3r, t3i = br + dr, bi + di, br - dr, bi - di
    lo = (t1r + t3i, t1i - t3r)
    hi = (t1r - t3i, t1i + t3r)
    if sign > 0:
        lo, hi = hi, lo
    return [(t0r + t2r, t0i + t2i), lo, (t0r - t2r, t0i - t2i), hi]


def _twiddle16(z, e, sign):
    zr, zi = z
    if e == 0:
        return z
    if e == 4:
        return (-zi, zr) if sign > 0 else (zi, -zr)
    h = float(np.sqrt(0.5))
    if e == 2:
        return ((zr - zi) * h, (zr + zi) * h) if sign > 0 else ((zr + zi) * h, (zi - zr) * h)
    if e == 6:
        return ((zr + zi) * -h, (zr - zi) * h) if sign > 0 else ((zi - zr) * h, (zr + zi) * -h)
    c = float(np.cos(2 * np.pi * e / 16))
    s = float(sign * np.sin(2 * np.pi * e / 16))
    return (zr * c - zi * s, zr * s + zi * c)


def _dft16(x, sign):
    cols = [_dft4([x[n1 + 4 * n2] for n2 in range(4)], sign) for n1 in range(4)]
    out = [None] * 16
    for k2 in range(4):
        res = _dft4([_twiddle16(cols[n1][k2], n1 * k2, sign) for n1 in range(4)], sign)
        for k1 in range(4):
            out[k2 + 4 * k1] = res[k1]
    return out


def _kernel(ax_hbm, mem_ref, wq_hbm, wk_hbm, wv_hbm, wo_hbm, bx_hbm, wr_hbm, wi_hbm,
            wrn_ref, win_ref, fd_hbm, tab_ref, out_hbm,
            wqkv, wo, ax, ao, bx, wr, wi, fd, cm, y, xa, qa, h_ref, ob_ref, acc_ref,
            sem_w, sem_m, sem_o):
    qkv_u32 = [w.bitcast(U32) for w in (wq_hbm, wk_hbm, wv_hbm)]
    wo_u32 = wo_hbm.bitcast(U32)
    bx_u32 = bx_hbm.bitcast(U32)
    out_u32 = out_hbm.bitcast(U32)

    def bx_copy(c):
        return pltpu.make_async_copy(bx_u32.at[:, c, :], bx.at[c], sem_m.at[6 + c])

    def slab_copy(j, hp):
        return pltpu.make_async_copy(qkv_u32[j].at[:, hp, :], wqkv.at[j * 16 + hp + 1],
                                     sem_w.at[j * 16 + hp])

    def repair(i):
        for g in range(8):
            ev = wqkv[i + 1, pl.ds(g * 128, 64, stride=2), :]
            od = wqkv[i + 1, pl.ds(g * 128 + 1, 64, stride=2), :]
            wqkv[i, g * 64:(g + 1) * 64, :] = (ev & jnp.uint32(0xFFFF)) | (od << 16)
            wqkv[i, 512 + g * 64:512 + (g + 1) * 64, :] = (
                (ev >> 16) | (od & jnp.uint32(0xFFFF0000)))

    early = 2
    cp_fd = pltpu.make_async_copy(fd_hbm, fd, sem_m.at[0])

    def w_copies(c):
        return [pltpu.make_async_copy(
            src.at[pl.ds(0, 512)].bitcast(U32).at[:, pl.ds(pl.multiple_of(m1 * 128, 128), 128)],
            dst.at[m1], sem_m.at[2])
            for src, dst in ((wr_hbm, wr), (wi_hbm, wi)) for m1 in (2 * c, 2 * c + 1)]

    def wo_copy(n):
        return pltpu.make_async_copy(wo_u32.at[:, pl.ds(pl.multiple_of(n * 128, 128), 128)],
                                     wo.at[n], sem_m.at[3])

    cp_lo = pltpu.make_async_copy(ax_hbm.at[:, 0], ax.at[:, 0], sem_m.at[1])
    cp_hi0, cp_hi1 = (
        pltpu.make_async_copy(ax_hbm.at[segs, pl.ds(1, 3)], ax.at[segs, pl.ds(1, 3)], sem_m.at[k])
        for segs, k in ((pl.ds(0, early), 4), (pl.ds(early, _NSEG - early), 5)))
    cp_fd.start()
    for c in range(3):
        bx_copy(c).start()
    for cp in w_copies(0):
        cp.start()

    h2 = float(np.sqrt(0.5))

    def half(u, par):
        u = (u << 16) if par == 0 else (u & jnp.uint32(0xFFFF0000))
        return lax.bitcast_convert_type(u, F32)

    def s_matrix(a, carry):
        c0, s0 = tab_ref[0:128, 0:128], tab_ref[0:128, 128:256]
        rows = pl.ds(pl.multiple_of(128 + 8 * a, 8), 8)
        tc, ts = tab_ref[rows, 0:128][0:1], tab_ref[rows, 128:256][0:1]
        cc, ss = c0 * tc - s0 * ts, c0 * ts + s0 * tc
        cm[a, 0:128, 0:128] = cc.astype(BF16)
        cm[a, 0:128, 128:256] = ss.astype(BF16)
        cm[a, 128:256, 0:128] = (-ss).astype(BF16)
        cm[a, 128:256, 128:256] = cc.astype(BF16)
        return carry

    lax.fori_loop(0, 16, s_matrix, 0)
    cp_fd.wait()

    def forward(c, carry):
        @pl.when(c < 5)
        def _():
            bx_copy(c + 3).start()

        @pl.when(c < 7)
        def _():
            for cp in w_copies(c + 1):
                cp.start()

        @pl.when(c >= 5)
        def _():
            slab_copy(0, c - 5).start()

        @pl.when(c == 5)
        def _():
            cp_lo.start()

        bx_copy(c).wait()
        for par in range(2):
            a = 2 * c + par
            x = [half(bx[c, :, t * 128:(t + 1) * 128], par) for t in range(8)]
            e0, e1, e2, e3 = x[0] + x[4], x[0] - x[4], x[2] + x[6], x[2] - x[6]
            o0, o1, o2, o3 = x[1] + x[5], x[1] - x[5], x[3] + x[7], x[3] - x[7]
            ee, oo = e0 + e2, o0 + o2
            p, q = (o1 - o3) * h2, (o1 + o3) * h2
            ts = ((e1 + p, -(e3 + q)), (e0 - e2, o2 - o0), (e1 - p, e3 - q))
            re, im = [], []
            for g in range(3):
                t = jnp.concatenate([ts[g][0].astype(BF16), ts[g][1].astype(BF16)], axis=1)
                r = lax.dot_general(fd[g * 256:(g + 1) * 256, :], t, _NT,
                                    preferred_element_type=F32)
                re.append(r[0:128])
                im.append(r[128:256])
            r = lax.dot_general(fd[768:896, 0:128], (ee - oo).astype(BF16), _NT,
                                preferred_element_type=F32)
            re.append(r[0:64])
            im.append(r[64:128])
            r = lax.dot_general(fd[896:1040, 0:128], (ee + oo).astype(BF16), _NT,
                                preferred_element_type=F32)
            re.append(r[0:72])
            im.append(r[72:144])
            for r0, r1, g0, g1 in ((0, 256, 0, 2), (256, _KR, 2, 5)):
                u = jnp.concatenate([jnp.concatenate(re[g0:g1], axis=0),
                                     jnp.concatenate(im[g0:g1], axis=0)], axis=1)
                y[a, r0:r1, :] = jnp.dot(u, cm[a], preferred_element_type=F32)
        return carry

    lax.fori_loop(0, 8, forward, 0)
    slab_copy(0, 3).start()
    for c in range(8):
        for cp in w_copies(c):
            cp.wait()

    def spectral(rows, filt):
        xf = _dft16([(y[a, rows, 0:128], y[a, rows, 128:256]) for a in range(16)], -1)
        v = []
        for m1 in range(16):
            (xr, xi), (fr, fi) = xf[m1], filt(m1)
            v.append((xr * fr - xi * fi, xr * fi + xi * fr))
        res = _dft16(v, +1)
        for a in range(16):
            y[a, rows, 0:128] = res[a][0]
            y[a, rows, 128:256] = res[a][1]

    cp_lo.wait()
    for g in range(8):
        xa[g * 64:(g + 1) * 64, :] = (
            ax[g * 8:(g + 1) * 8, 0, :, :].astype(F32).reshape(64, _D))
    slab_copy(0, 0).wait()
    repair(0)

    def middle(i, carry):
        @pl.when(i < 12)
        def _():
            slab_copy(0, i + 4).start()

        slab_copy(1, i).start()
        slab_copy(2, i).start()
        slab_copy(0, i + 1).wait()
        c = i // 4
        for par in range(2):
            w = pltpu.bitcast(wqkv[i, par * 512:(par + 1) * 512, :], BF16)
            blk = _RES.index(par)
            for cc in range(1, 4):
                blk = jnp.where(c == cc, _RES.index(2 * cc + par), blk)
            for k in range(2):
                qa[2 * i + par, k * 256:(k + 1) * 256] = jnp.dot(
                    xa[k * 256:(k + 1) * 256], w, preferred_element_type=F32)
                jg = 2 * (i % 4) + k
                w_rows = pl.ds(jg * 32 + c, 8, stride=4)
                spectral(pl.ds(pl.multiple_of(blk * 64 + jg * 8, 8), 8),
                         lambda m1: (half(wr[m1, w_rows, :], par), half(wi[m1, w_rows, :], par)))
        repair(i + 1)
        return carry

    lax.fori_loop(0, 16, middle, 0)
    spectral(pl.ds(512, 8),
             lambda m1: tuple(jnp.broadcast_to(w[0:1, m1 * 128:(m1 + 1) * 128].astype(F32), (8, 128))
                             for w in (wrn_ref, win_ref)))

    sign = jnp.where(lax.broadcasted_iota(jnp.int32, (128, 256), 0) % 2 == 0, 1.0, -1.0)

    def b_out_copy(c):
        return pltpu.make_async_copy(bx.at[c], out_u32.at[:, c, pl.ds(_D, _D)], sem_o.at[0])

    def inverse(c, carry):
        @pl.when(c < 4)
        def _():
            wo_copy(2 * c).start()
            wo_copy(2 * c + 1).start()

        slab_copy(0, 17 + 2 * c).wait()
        slab_copy(0, 18 + 2 * c).wait()
        zs = {}
        for par in range(2):
            a = 2 * c + par
            for g in range(4):
                z = lax.dot_general(cm[a], y[a, g * 128:(g + 1) * 128, :].astype(BF16), _NT,
                                    preferred_element_type=F32)
                zr, zi = z[0:128], z[128:256]
                if g < 3:
                    zs[par, g] = jnp.concatenate([zr, zi], axis=1).astype(BF16)
                else:
                    low = lax.broadcasted_iota(jnp.int32, (128, 128), 1) < 64
                    zs[par, 3] = jnp.where(low, zr, pltpu.roll(zi, 64, 1)).astype(BF16)
                    zs[par, 4] = jnp.where(low, pltpu.roll(zr, 64, 1), zi).astype(BF16)
            zs[par, 5] = lax.dot_general(
                cm[a, 0:128, :], (y[a, 512:513, :] * sign).astype(BF16), _NT,
                preferred_element_type=F32)
        outs = []
        for par in range(2):
            qs = []
            for g in range(3):
                r = jnp.dot(zs[par, g], fd[g * 256:(g + 1) * 256, :],
                            preferred_element_type=F32)
                qs.append((r[:, 0:128], r[:, 128:256]))
            (q1r, q1i), (q2r, q2i), (q3r, q3i) = qs
            r4 = jnp.dot(zs[par, 3], fd[768:896, 0:128], preferred_element_type=F32)
            r0 = jnp.dot(zs[par, 4], fd[768:896, 128:256],
                         preferred_element_type=F32) + zs[par, 5]
            ee, oo = r0 + r4, r0 - r4
            e0, e2, o0, o2 = ee + q2r, ee - q2r, oo - q2i, oo + q2i
            e1, e3 = q1r + q3r, q3i - q1i
            p, q = (q1r - q3r) * h2, (q1i + q3i) * h2
            o1, o3 = p - q, -(p + q)
            cols = (e0 + e1, o0 + o1, e2 + e3, o2 + o3, e0 - e1, o0 - o1, e2 - e3, o2 - o3)
            outs.append([lax.bitcast_convert_type(v.astype(BF16).astype(F32), U32)
                         for v in cols])
        for t in range(8):
            bx[c, :, t * 128:(t + 1) * 128] = (outs[0][t] >> 16) | outs[1][t]
        repair(17 + 2 * c)
        repair(18 + 2 * c)
        return carry

    cp_hi0.start()
    lax.fori_loop(0, 8, inverse, 0)

    def last_slabs(i, carry):
        slab_copy(0, i).wait()
        repair(i)
        return carry

    lax.fori_loop(33, 48, last_slabs, 0)
    cp_hi0.wait()
    for n in range(8):
        wo_copy(n).wait()
    cp_hi1.start()

    def position(i):
        return jnp.where(i < 8, i + _M, jnp.where(i < 8 + _M, i - 8, i))

    qi = position(lax.broadcasted_iota(jnp.int32, (_L, _L), 0))
    ki = position(lax.broadcasted_iota(jnp.int32, (_L, _L), 1))
    mask = (qi < _M) | (qi >= ki)
    scale = 128 ** -0.5
    group, skew, lag, slag, order = 8, 1, 2, 1, 'kqsvop'
    n_group = _H // group

    def load_tokens(s):
        for k, r0 in enumerate((0, 16, 24, 32)):
            h_ref[r0:r0 + 8, :] = ax[s, k].astype(F32)

    h_ref[8:16, :] = mem_ref[...].astype(F32)
    load_tokens(0)

    def a_out_copy(s):
        rows = pl.ds(2 * s, 2)
        return pltpu.make_async_copy(ao.at[rows], out_hbm.at[rows, :, pl.ds(0, _D)],
                                     sem_o.at[1])

    def step(s, carry):
        st = {}

        def proj(j, hd):
            w = wqkv[j * 16 + hd // 2, (hd % 2) * 512:(hd % 2 + 1) * 512, :]
            r = jnp.dot(h_ref[(8 if j == 0 else 0):_L, :], pltpu.bitcast(w, BF16),
                        preferred_element_type=F32)
            if j == 0:
                r = jnp.concatenate([qa[hd, pl.ds(pl.multiple_of(s * 8, 8), 8), :], r], axis=0)
            st[j, hd] = r

        def scores(hd):
            sc = lax.dot_general(st[0, hd], st[1, hd], _NT, preferred_element_type=F32) * scale
            sc = jnp.where(mask, sc, -1000000000.0)
            p = jnp.exp(sc - jnp.max(sc, axis=1, keepdims=True))
            st['p', hd] = p
            st['l', hd] = 1.0 / jnp.sum(p, axis=1, keepdims=True)

        def pv(hd):
            o = jnp.dot(st['p', hd], st[2, hd], preferred_element_type=F32)
            ob_ref[:, hd * 128:(hd + 1) * 128] = o * st['l', hd]

        def w_out(g, n):
            lanes = slice(n * 128, (n + 1) * 128)
            w = wo[n, g * group * 64:(g + 1) * group * 64, :]
            r = jnp.dot(ob_ref[:, g * group * 128:(g + 1) * group * 128],
                        pltpu.bitcast(w, BF16), preferred_element_type=F32)
            if g > 0:
                r = r + acc_ref[:, lanes]
            if g < n_group - 1:
                acc_ref[:, lanes] = r
            else:
                h_ref[8:16, lanes] = r[8:16].astype(BF16).astype(F32)
                ao[2 * s, :, lanes] = jnp.concatenate([r[0:8], r[16:24]], axis=0).astype(BF16)
                ao[2 * s + 1, :, lanes] = r[24:40].astype(BF16)

        def next_x():
            load_tokens(jnp.minimum(s + 1, _NSEG - 1))

        ops, pending = [], []
        for t in range(_H + skew + lag + slag):
            for what in order:
                if what == 'q' and t < _H:
                    ops.append((proj, 0, t))
                if what == 'k' and t < _H:
                    ops.append((proj, 1, t))
                if what == 's' and 0 <= t - slag < _H:
                    ops.append((scores, t - slag))
                if what == 'o' and pending:
                    ops.append(pending.pop(0))
                if what == 'v' and 0 <= t - skew < _H:
                    ops.append((proj, 2, t - skew))
                    if t - skew == _H - 1:
                        ops.append((next_x,))
                hd = t - skew - lag
                if what == 'p' and 0 <= hd < _H:
                    if hd == _H - 1:
                        ops += pending
                        pending = []
                    ops.append((pv, hd))
                    if hd % group == group - 1:
                        pending += [(w_out, hd // group, n) for n in range(8)]
        ops += pending
        for op in ops:
            op[0](*op[1:])
        a_out_copy(s).start()
        return carry

    def segments(part, carry):
        lax.fori_loop(part * early, early + part * (_NSEG - early), step, 0)

        @pl.when(part == 0)
        def _():
            cp_hi1.wait()
            for c in range(8):
                b_out_copy(c).start()

        return carry

    lax.fori_loop(0, 2, segments, 0)

    def drain_b(a, carry):
        b_out_copy(a).wait()
        return carry

    def drain_a(s, carry):
        a_out_copy(s).wait()
        return carry

    lax.fori_loop(0, 8, drain_b, 0)
    lax.fori_loop(0, _NSEG, drain_a, 0)


@jax.jit
def _run(A_x, A_mem0, A_Wq, A_Wk, A_Wv, A_Wo, B_x, B_w_r, B_w_i):
    hbm = pl.BlockSpec(memory_space=pltpu.HBM)
    vmem = pl.BlockSpec(memory_space=pltpu.VMEM)
    nyquist = pl.BlockSpec((16, _S), lambda i: (512 // 16, 0))
    wr, wi = B_w_r.T, B_w_i.T
    out = pl.pallas_call(
        _kernel,
        grid=(1,),
        out_shape=jax.ShapeDtypeStruct((128, 16, 2 * _D), BF16),
        in_specs=[hbm, vmem, hbm, hbm, hbm, hbm, hbm, hbm, hbm, nyquist, nyquist, hbm, vmem],
        out_specs=hbm,
        scratch_shapes=[
            pltpu.VMEM((49, 1024, 128), U32),
            pltpu.VMEM((8, 2048, 128), U32),
            pltpu.VMEM((_NSEG, 4, 8, _D), BF16),
            pltpu.VMEM((128, 16, _D), BF16),
            pltpu.VMEM((8, 128, _D), U32),
            pltpu.VMEM((16, 256, 128), U32),
            pltpu.VMEM((16, 256, 128), U32),
            pltpu.VMEM((1040, 256), BF16),
            pltpu.VMEM((16, 256, 256), BF16),
            pltpu.VMEM((16, _KR, 256), F32),
            pltpu.VMEM((_NSEG * 8, _D), F32),
            pltpu.VMEM((_H, _NSEG * 8, 128), F32),
            pltpu.VMEM((_L, _D), F32),
            pltpu.VMEM((_L, _H * 128), F32),
            pltpu.VMEM((_L, _D), F32),
            pltpu.SemaphoreType.DMA((48,)),
            pltpu.SemaphoreType.DMA((14,)),
            pltpu.SemaphoreType.DMA((2,)),
        ],
        compiler_params=pltpu.CompilerParams(vmem_limit_bytes=100 * 1024 * 1024),
    )(A_x.reshape(_NSEG, 4, 8, _D), A_mem0.reshape(_M, _D), A_Wq, A_Wk, A_Wv,
      A_Wo.reshape(_H * 128, _D), B_x.reshape(128, 16, _D), wr, wi, wr, wi, *_CONSTS)
    return out.reshape(1, _S, 2 * _D)


def pallas_concat_heads__memory_aug_recurrent_mem_tr__spectral_gfnet__prompt_kernel(
    A_x, A_mem0, A_Wq, A_Wk, A_Wv, A_Wo, A_seg_len, B_x, B_w_r, B_w_i,
):
    assert int(A_seg_len) == _SEG
    return _run(A_x, A_mem0, A_Wq, A_Wk, A_Wv, A_Wo, B_x, B_w_r, B_w_i)
```

```python
import numpy as np

import jax
import jax.numpy as jnp
from jax import lax
import jax.experimental.pallas as pl
import jax.experimental.pallas.tpu as pltpu

F32 = jnp.float32
BF16 = jnp.bfloat16
U32 = jnp.uint32

_S = 2048
_D = 1024
_H = 32
_M = 8
_SEG = 32
_L = _M + _SEG
_NSEG = _S // _SEG
_KR = 520
_NK = 3
_RES = (1, 7, 2, 6, 3, 5, 4, 0)

_NT = (((1,), (1,)), ((), ()))


def _dft_constants():
    b = np.arange(128)

    def cs(k):
        ang = -2.0 * np.pi * ((k[:, None] * b[None, :]) % _D) / _D
        return np.cos(ang), np.sin(ang)

    j = np.arange(64)
    fd = np.zeros((1040, 256))
    for g, r in enumerate((1, 2, 3)):
        c1, s1 = cs(r + 8 * j)
        c2, s2 = cs(8 - r + 8 * j)
        fd[g * 256:(g + 1) * 256] = np.block([[c1, -s1], [c2, s2], [s1, c1], [s2, -c2]])
    c4, s4 = cs(4 + 8 * j)
    fd[768:896, :128] = np.concatenate([c4, s4], 0)
    c0, s0 = cs(8 * np.arange(72))
    c0[65:] = 0.0
    s0[64:] = 0.0
    s0[0] = 0.0
    fd[768:896, 128:] = np.concatenate([c0[:64], s0[:64]], 0)
    c0[0] *= 0.5
    c0[64] *= 0.5
    fd[896:1040, :128] = np.concatenate([c0, s0], 0)

    ang = -2.0 * np.pi * ((b[:, None] * b[None, :]) % 128) / 128
    tw = -2.0 * np.pi * ((np.arange(128) // 8)[:, None] * b[None, :]) / _S
    norm = np.sqrt(2.0 / (_S * _D))
    tab = np.block([[np.cos(ang), np.sin(ang)], [np.cos(tw) * norm, np.sin(tw) * norm]])
    return np.asarray(fd, np.float32).astype(BF16), np.asarray(tab, np.float32)


_CONSTS = _dft_constants()


def _dft4(x, sign):
    (ar, ai), (br, bi), (cr, ci), (dr, di) = x
    t0r, t0i, t1r, t1i = ar + cr, ai + ci, ar - cr, ai - ci
    t2r, t2i, t3r, t3i = br + dr, bi + di, br - dr, bi - di
    lo = (t1r + t3i, t1i - t3r)
    hi = (t1r - t3i, t1i + t3r)
    if sign > 0:
        lo, hi = hi, lo
    return [(t0r + t2r, t0i + t2i), lo, (t0r - t2r, t0i - t2i), hi]


def _twiddle16(z, e, sign):
    zr, zi = z
    if e == 0:
        return z
    if e == 4:
        return (-zi, zr) if sign > 0 else (zi, -zr)
    h = float(np.sqrt(0.5))
    if e == 2:
        return ((zr - zi) * h, (zr + zi) * h) if sign > 0 else ((zr + zi) * h, (zi - zr) * h)
    if e == 6:
        return ((zr + zi) * -h, (zr - zi) * h) if sign > 0 else ((zi - zr) * h, (zr + zi) * -h)
    c = float(np.cos(2 * np.pi * e / 16))
    s = float(sign * np.sin(2 * np.pi * e / 16))
    return (zr * c - zi * s, zr * s + zi * c)


def _dft16(x, sign):
    cols = [_dft4([x[n1 + 4 * n2] for n2 in range(4)], sign) for n1 in range(4)]
    out = [None] * 16
    for k2 in range(4):
        res = _dft4([_twiddle16(cols[n1][k2], n1 * k2, sign) for n1 in range(4)], sign)
        for k1 in range(4):
            out[k2 + 4 * k1] = res[k1]
    return out


def _kernel(ax_hbm, mem_ref, wq_hbm, wk_hbm, wv_hbm, wo_hbm, bx_hbm, wr_hbm, wi_hbm,
            wrn_ref, win_ref, fd_hbm, tab_ref, out_hbm,
            wqkv, wo, ax, ao, bx, wr, wi, fd, cm, y, xa, qa, h_ref, ob_ref, acc_ref,
            sem_w, sem_m, sem_o):
    qkv_u32 = [w.bitcast(U32) for w in (wq_hbm, wk_hbm, wv_hbm)]
    wo_u32 = wo_hbm.bitcast(U32)
    bx_u32 = bx_hbm.bitcast(U32)
    out_u32 = out_hbm.bitcast(U32)

    def bx_copy(c):
        return pltpu.make_async_copy(bx_u32.at[:, c, :], bx.at[c], sem_m.at[6 + c])

    def slab_copy(j, hp):
        return pltpu.make_async_copy(qkv_u32[j].at[:, hp, :], wqkv.at[j * 16 + hp + 1],
                                     sem_w.at[j * 16 + hp])

    def repair(i):
        for g in range(8):
            ev = wqkv[i + 1, pl.ds(g * 128, 64, stride=2), :]
            od = wqkv[i + 1, pl.ds(g * 128 + 1, 64, stride=2), :]
            wqkv[i, g * 64:(g + 1) * 64, :] = (ev & jnp.uint32(0xFFFF)) | (od << 16)
            wqkv[i, 512 + g * 64:512 + (g + 1) * 64, :] = (
                (ev >> 16) | (od & jnp.uint32(0xFFFF0000)))

    early = 2
    cp_fd = pltpu.make_async_copy(fd_hbm, fd, sem_m.at[0])

    def w_copies(c):
        return [pltpu.make_async_copy(
            src.at[pl.ds(0, 512)].bitcast(U32).at[:, pl.ds(pl.multiple_of(m1 * 128, 128), 128)],
            dst.at[m1], sem_m.at[2])
            for src, dst in ((wr_hbm, wr), (wi_hbm, wi)) for m1 in (2 * c, 2 * c + 1)]

    def wo_copy(n):
        return pltpu.make_async_copy(wo_u32.at[:, pl.ds(pl.multiple_of(n * 128, 128), 128)],
                                     wo.at[n], sem_m.at[3])

    cp_lo = pltpu.make_async_copy(ax_hbm.at[:, 0], ax.at[:, 0], sem_m.at[1])
    cp_hi0, cp_hi1 = (
        pltpu.make_async_copy(ax_hbm.at[segs, pl.ds(1, 3)], ax.at[segs, pl.ds(1, 3)], sem_m.at[k])
        for segs, k in ((pl.ds(0, early), 4), (pl.ds(early, _NSEG - early), 5)))
    cp_fd.start()
    for c in range(3):
        bx_copy(c).start()
    for cp in w_copies(0):
        cp.start()

    h2 = float(np.sqrt(0.5))

    def half(u, par):
        u = (u << 16) if par == 0 else (u & jnp.uint32(0xFFFF0000))
        return lax.bitcast_convert_type(u, F32)

    def s_matrix(a, carry):
        c0, s0 = tab_ref[0:128, 0:128], tab_ref[0:128, 128:256]
        rows = pl.ds(pl.multiple_of(128 + 8 * a, 8), 8)
        tc, ts = tab_ref[rows, 0:128][0:1], tab_ref[rows, 128:256][0:1]
        cc, ss = c0 * tc - s0 * ts, c0 * ts + s0 * tc
        cm[a, 0:128, 0:128] = cc.astype(BF16)
        cm[a, 0:128, 128:256] = ss.astype(BF16)
        cm[a, 128:256, 0:128] = (-ss).astype(BF16)
        cm[a, 128:256, 128:256] = cc.astype(BF16)
        return carry

    lax.fori_loop(0, 16, s_matrix, 0)
    cp_fd.wait()

    def forward(c, carry):
        @pl.when(c < 5)
        def _():
            bx_copy(c + 3).start()

        @pl.when(c < 7)
        def _():
            for cp in w_copies(c + 1):
                cp.start()

        @pl.when(c >= 5)
        def _():
            slab_copy(0, c - 5).start()

        @pl.when(c == 5)
        def _():
            cp_lo.start()

        bx_copy(c).wait()
        for par in range(2):
            a = 2 * c + par
            x = [half(bx[c, :, t * 128:(t + 1) * 128], par) for t in range(8)]
            e0, e1, e2, e3 = x[0] + x[4], x[0] - x[4], x[2] + x[6], x[2] - x[6]
            o0, o1, o2, o3 = x[1] + x[5], x[1] - x[5], x[3] + x[7], x[3] - x[7]
            ee, oo = e0 + e2, o0 + o2
            p, q = (o1 - o3) * h2, (o1 + o3) * h2
            ts = ((e1 + p, -(e3 + q)), (e0 - e2, o2 - o0), (e1 - p, e3 - q))
            re, im = [], []
            for g in range(3):
                t = jnp.concatenate([ts[g][0].astype(BF16), ts[g][1].astype(BF16)], axis=1)
                r = lax.dot_general(fd[g * 256:(g + 1) * 256, :], t, _NT,
                                    preferred_element_type=F32)
                re.append(r[0:128])
                im.append(r[128:256])
            r = lax.dot_general(fd[768:896, 0:128], (ee - oo).astype(BF16), _NT,
                                preferred_element_type=F32)
            re.append(r[0:64])
            im.append(r[64:128])
            r = lax.dot_general(fd[896:1040, 0:128], (ee + oo).astype(BF16), _NT,
                                preferred_element_type=F32)
            re.append(r[0:72])
            im.append(r[72:144])
            for r0, r1, g0, g1 in ((0, 256, 0, 2), (256, _KR, 2, 5)):
                u = jnp.concatenate([jnp.concatenate(re[g0:g1], axis=0),
                                     jnp.concatenate(im[g0:g1], axis=0)], axis=1)
                y[a, r0:r1, :] = jnp.dot(u, cm[a], preferred_element_type=F32)
        return carry

    lax.fori_loop(0, 8, forward, 0)
    slab_copy(0, 3).start()
    for c in range(8):
        for cp in w_copies(c):
            cp.wait()

    def spectral(rows, filt):
        xf = _dft16([(y[a, rows, 0:128], y[a, rows, 128:256]) for a in range(16)], -1)
        v = []
        for m1 in range(16):
            (xr, xi), (fr, fi) = xf[m1], filt(m1)
            v.append((xr * fr - xi * fi, xr * fi + xi * fr))
        res = _dft16(v, +1)
        for a in range(16):
            y[a, rows, 0:128] = res[a][0]
            y[a, rows, 128:256] = res[a][1]

    cp_lo.wait()
    for g in range(8):
        xa[g * 64:(g + 1) * 64, :] = (
            ax[g * 8:(g + 1) * 8, 0, :, :].astype(F32).reshape(64, _D))
    slab_copy(0, 0).wait()
    repair(0)

    def middle(i, carry):
        @pl.when(i < 12)
        def _():
            slab_copy(0, i + 4).start()

        slab_copy(1, i).start()

        @pl.when(i % 4 != 3)
        def _():
            slab_copy(2, i - i // 4).start()

        slab_copy(0, i + 1).wait()
        repair(i + 1)
        c = i // 4
        for par in range(2):
            w = pltpu.bitcast(wqkv[i, par * 512:(par + 1) * 512, :], BF16)
            blk = _RES.index(par)
            for cc in range(1, 4):
                blk = jnp.where(c == cc, _RES.index(2 * cc + par), blk)
            for k in range(2):
                qa[2 * i + par, k * 256:(k + 1) * 256] = jnp.dot(
                    xa[k * 256:(k + 1) * 256], w, preferred_element_type=F32)
                jg = 2 * (i % 4) + k
                w_rows = pl.ds(jg * 32 + c, 8, stride=4)
                spectral(pl.ds(pl.multiple_of(blk * 64 + jg * 8, 8), 8),
                         lambda m1: (half(wr[m1, w_rows, :], par), half(wi[m1, w_rows, :], par)))
        return carry

    lax.fori_loop(0, 16, middle, 0)
    spectral(pl.ds(512, 8),
             lambda m1: tuple(jnp.broadcast_to(w[0:1, m1 * 128:(m1 + 1) * 128].astype(F32), (8, 128))
                             for w in (wrn_ref, win_ref)))

    sign = jnp.where(lax.broadcasted_iota(jnp.int32, (128, 256), 0) % 2 == 0, 1.0, -1.0)

    def b_out_copy(c):
        return pltpu.make_async_copy(bx.at[c], out_u32.at[:, c, pl.ds(_D, _D)], sem_o.at[0])

    def inverse(c, carry):
        @pl.when(c < 4)
        def _():
            wo_copy(2 * c).start()
            wo_copy(2 * c + 1).start()

        slab_copy(0, 17 + 2 * c).wait()
        slab_copy(0, 18 + 2 * c).wait()
        zs = {}
        for par in range(2):
            a = 2 * c + par
            for g in range(4):
                z = lax.dot_general(cm[a], y[a, g * 128:(g + 1) * 128, :].astype(BF16), _NT,
                                    preferred_element_type=F32)
                zr, zi = z[0:128], z[128:256]
                if g < 3:
                    zs[par, g] = jnp.concatenate([zr, zi], axis=1).astype(BF16)
                else:
                    low = lax.broadcasted_iota(jnp.int32, (128, 128), 1) < 64
                    zs[par, 3] = jnp.where(low, zr, pltpu.roll(zi, 64, 1)).astype(BF16)
                    zs[par, 4] = jnp.where(low, pltpu.roll(zr, 64, 1), zi).astype(BF16)
            zs[par, 5] = lax.dot_general(
                cm[a, 0:128, :], (y[a, 512:513, :] * sign).astype(BF16), _NT,
                preferred_element_type=F32)
        outs = []
        for par in range(2):
            qs = []
            for g in range(3):
                r = jnp.dot(zs[par, g], fd[g * 256:(g + 1) * 256, :],
                            preferred_element_type=F32)
                qs.append((r[:, 0:128], r[:, 128:256]))
            (q1r, q1i), (q2r, q2i), (q3r, q3i) = qs
            r4 = jnp.dot(zs[par, 3], fd[768:896, 0:128], preferred_element_type=F32)
            r0 = jnp.dot(zs[par, 4], fd[768:896, 128:256],
                         preferred_element_type=F32) + zs[par, 5]
            ee, oo = r0 + r4, r0 - r4
            e0, e2, o0, o2 = ee + q2r, ee - q2r, oo - q2i, oo + q2i
            e1, e3 = q1r + q3r, q3i - q1i
            p, q = (q1r - q3r) * h2, (q1i + q3i) * h2
            o1, o3 = p - q, -(p + q)
            cols = (e0 + e1, o0 + o1, e2 + e3, o2 + o3, e0 - e1, o0 - o1, e2 - e3, o2 - o3)
            outs.append([lax.bitcast_convert_type(v.astype(BF16).astype(F32), U32)
                         for v in cols])
        for t in range(8):
            bx[c, :, t * 128:(t + 1) * 128] = (outs[0][t] >> 16) | outs[1][t]
        repair(17 + 2 * c)
        repair(18 + 2 * c)
        return carry

    for hp in range(12, 16):
        slab_copy(2, hp).start()
    cp_hi0.start()
    lax.fori_loop(0, 8, inverse, 0)

    def last_slabs(i, carry):
        slab_copy(0, i).wait()
        repair(i)
        return carry

    lax.fori_loop(33, 48, last_slabs, 0)
    for hd in range(_NK):
        w = pltpu.bitcast(wqkv[16 + hd // 2, (hd % 2) * 512:(hd % 2 + 1) * 512, :], BF16)
        qa[_H + hd] = jnp.dot(xa[...], w, preferred_element_type=F32)
    cp_hi0.wait()
    for n in range(8):
        wo_copy(n).wait()
    cp_hi1.start()

    def position(i):
        return jnp.where(i < 8, i + _M, jnp.where(i < 8 + _M, i - 8, i))

    qi = position(lax.broadcasted_iota(jnp.int32, (_L, _L), 0))
    ki = position(lax.broadcasted_iota(jnp.int32, (_L, _L), 1))
    mask = (qi < _M) | (qi >= ki)
    scale = 128 ** -0.5
    group, skew, lag, slag, order = 8, 1, 2, 1, 'kqsvop'
    n_group = _H // group

    def load_tokens(s):
        for k, r0 in enumerate((0, 16, 24, 32)):
            h_ref[r0:r0 + 8, :] = ax[s, k].astype(F32)

    h_ref[8:16, :] = mem_ref[...].astype(F32)
    load_tokens(0)

    def a_out_copy(s):
        rows = pl.ds(2 * s, 2)
        return pltpu.make_async_copy(ao.at[rows], out_hbm.at[rows, :, pl.ds(0, _D)],
                                     sem_o.at[1])

    def step(s, carry):
        st = {}

        def proj(j, hd):
            w = wqkv[j * 16 + hd // 2, (hd % 2) * 512:(hd % 2 + 1) * 512, :]
            hoisted = j * _H + hd < _H + _NK
            r = jnp.dot(h_ref[(8 if hoisted else 0):_L, :], pltpu.bitcast(w, BF16),
                        preferred_element_type=F32)
            if hoisted:
                r = jnp.concatenate(
                    [qa[j * _H + hd, pl.ds(pl.multiple_of(s * 8, 8), 8), :], r], axis=0)
            st[j, hd] = r

        def scores(hd):
            sc = lax.dot_general(st[0, hd], st[1, hd], _NT, preferred_element_type=F32) * scale
            sc = jnp.where(mask, sc, -1000000000.0)
            p = jnp.exp(sc - jnp.max(sc, axis=1, keepdims=True))
            st['p', hd] = p
            st['l', hd] = 1.0 / jnp.sum(p, axis=1, keepdims=True)

        def pv(hd):
            o = jnp.dot(st['p', hd], st[2, hd], preferred_element_type=F32)
            ob_ref[:, hd * 128:(hd + 1) * 128] = o * st['l', hd]

        def w_out(g, n):
            lanes = slice(n * 128, (n + 1) * 128)
            w = wo[n, g * group * 64:(g + 1) * group * 64, :]
            r = jnp.dot(ob_ref[:, g * group * 128:(g + 1) * group * 128],
                        pltpu.bitcast(w, BF16), preferred_element_type=F32)
            if g > 0:
                r = r + acc_ref[:, lanes]
            if g < n_group - 1:
                acc_ref[:, lanes] = r
            else:
                h_ref[8:16, lanes] = r[8:16].astype(BF16).astype(F32)
                ao[2 * s, :, lanes] = jnp.concatenate([r[0:8], r[16:24]], axis=0).astype(BF16)
                ao[2 * s + 1, :, lanes] = r[24:40].astype(BF16)

        def next_x():
            load_tokens(jnp.minimum(s + 1, _NSEG - 1))

        ops, pending = [], []
        for t in range(_H + skew + lag + slag):
            for what in order:
                if what == 'q' and t < _H:
                    ops.append((proj, 0, t))
                if what == 'k' and t < _H:
                    ops.append((proj, 1, t))
                if what == 's' and 0 <= t - slag < _H:
                    ops.append((scores, t - slag))
                if what == 'o' and pending:
                    ops.append(pending.pop(0))
                if what == 'v' and 0 <= t - skew < _H:
                    ops.append((proj, 2, t - skew))
                    if t - skew == _H - 1:
                        ops.append((next_x,))
                hd = t - skew - lag
                if what == 'p' and 0 <= hd < _H:
                    if hd == _H - 1:
                        ops += pending
                        pending = []
                    ops.append((pv, hd))
                    if hd % group == group - 1:
                        pending += [(w_out, hd // group, n) for n in range(8)]
        ops += pending
        for op in ops:
            op[0](*op[1:])
        a_out_copy(s).start()
        return carry

    def segments(part, carry):
        lax.fori_loop(part * early, early + part * (_NSEG - early), step, 0)

        @pl.when(part == 0)
        def _():
            cp_hi1.wait()
            for c in range(8):
                b_out_copy(c).start()

        return carry

    lax.fori_loop(0, 2, segments, 0)

    def drain_b(a, carry):
        b_out_copy(a).wait()
        return carry

    def drain_a(s, carry):
        a_out_copy(s).wait()
        return carry

    lax.fori_loop(0, 8, drain_b, 0)
    lax.fori_loop(0, _NSEG, drain_a, 0)


@jax.jit
def _run(A_x, A_mem0, A_Wq, A_Wk, A_Wv, A_Wo, B_x, B_w_r, B_w_i):
    hbm = pl.BlockSpec(memory_space=pltpu.HBM)
    vmem = pl.BlockSpec(memory_space=pltpu.VMEM)
    nyquist = pl.BlockSpec((16, _S), lambda i: (512 // 16, 0))
    wr, wi = B_w_r.T, B_w_i.T
    out = pl.pallas_call(
        _kernel,
        grid=(1,),
        out_shape=jax.ShapeDtypeStruct((128, 16, 2 * _D), BF16),
        in_specs=[hbm, vmem, hbm, hbm, hbm, hbm, hbm, hbm, hbm, nyquist, nyquist, hbm, vmem],
        out_specs=hbm,
        scratch_shapes=[
            pltpu.VMEM((49, 1024, 128), U32),
            pltpu.VMEM((8, 2048, 128), U32),
            pltpu.VMEM((_NSEG, 4, 8, _D), BF16),
            pltpu.VMEM((128, 16, _D), BF16),
            pltpu.VMEM((8, 128, _D), U32),
            pltpu.VMEM((16, 256, 128), U32),
            pltpu.VMEM((16, 256, 128), U32),
            pltpu.VMEM((1040, 256), BF16),
            pltpu.VMEM((16, 256, 256), BF16),
            pltpu.VMEM((16, _KR, 256), F32),
            pltpu.VMEM((_NSEG * 8, _D), F32),
            pltpu.VMEM((_H + _NK, _NSEG * 8, 128), F32),
            pltpu.VMEM((_L, _D), F32),
            pltpu.VMEM((_L, _H * 128), F32),
            pltpu.VMEM((_L, _D), F32),
            pltpu.SemaphoreType.DMA((48,)),
            pltpu.SemaphoreType.DMA((14,)),
            pltpu.SemaphoreType.DMA((2,)),
        ],
        compiler_params=pltpu.CompilerParams(vmem_limit_bytes=100 * 1024 * 1024),
    )(A_x.reshape(_NSEG, 4, 8, _D), A_mem0.reshape(_M, _D), A_Wq, A_Wk, A_Wv,
      A_Wo.reshape(_H * 128, _D), B_x.reshape(128, 16, _D), wr, wi, wr, wi, *_CONSTS)
    return out.reshape(1, _S, 2 * _D)


def pallas_concat_heads__memory_aug_recurrent_mem_tr__spectral_gfnet__prompt_kernel(
    A_x, A_mem0, A_Wq, A_Wk, A_Wv, A_Wo, A_seg_len, B_x, B_w_r, B_w_i,
):
    assert int(A_seg_len) == _SEG
    return _run(A_x, A_mem0, A_Wq, A_Wk, A_Wv, A_Wo, B_x, B_w_r, B_w_i)
```

```python
import numpy as np

import jax
import jax.numpy as jnp
from jax import lax
import jax.experimental.pallas as pl
import jax.experimental.pallas.tpu as pltpu

F32 = jnp.float32
BF16 = jnp.bfloat16
U32 = jnp.uint32

_S = 2048
_D = 1024
_H = 32
_M = 8
_SEG = 32
_L = _M + _SEG
_NSEG = _S // _SEG
_KR = 520
_NK = 4
_RES = (1, 7, 2, 6, 3, 5, 4, 0)

_NT = (((1,), (1,)), ((), ()))


def _dft_constants():
    b = np.arange(128)

    def cs(k):
        ang = -2.0 * np.pi * ((k[:, None] * b[None, :]) % _D) / _D
        return np.cos(ang), np.sin(ang)

    j = np.arange(64)
    fd = np.zeros((1040, 256))
    for g, r in enumerate((1, 2, 3)):
        c1, s1 = cs(r + 8 * j)
        c2, s2 = cs(8 - r + 8 * j)
        fd[g * 256:(g + 1) * 256] = np.block([[c1, -s1], [c2, s2], [s1, c1], [s2, -c2]])
    c4, s4 = cs(4 + 8 * j)
    fd[768:896, :128] = np.concatenate([c4, s4], 0)
    c0, s0 = cs(8 * np.arange(72))
    c0[65:] = 0.0
    s0[64:] = 0.0
    s0[0] = 0.0
    fd[768:896, 128:] = np.concatenate([c0[:64], s0[:64]], 0)
    c0[0] *= 0.5
    c0[64] *= 0.5
    fd[896:1040, :128] = np.concatenate([c0, s0], 0)

    ang = -2.0 * np.pi * ((b[:, None] * b[None, :]) % 128) / 128
    tw = -2.0 * np.pi * ((np.arange(128) // 8)[:, None] * b[None, :]) / _S
    norm = np.sqrt(2.0 / (_S * _D))
    tab = np.block([[np.cos(ang), np.sin(ang)], [np.cos(tw) * norm, np.sin(tw) * norm]])
    return np.asarray(fd, np.float32).astype(BF16), np.asarray(tab, np.float32)


_CONSTS = _dft_constants()


def _dft4(x, sign):
    (ar, ai), (br, bi), (cr, ci), (dr, di) = x
    t0r, t0i, t1r, t1i = ar + cr, ai + ci, ar - cr, ai - ci
    t2r, t2i, t3r, t3i = br + dr, bi + di, br - dr, bi - di
    lo = (t1r + t3i, t1i - t3r)
    hi = (t1r - t3i, t1i + t3r)
    if sign > 0:
        lo, hi = hi, lo
    return [(t0r + t2r, t0i + t2i), lo, (t0r - t2r, t0i - t2i), hi]


def _twiddle16(z, e, sign):
    zr, zi = z
    if e == 0:
        return z
    if e == 4:
        return (-zi, zr) if sign > 0 else (zi, -zr)
    h = float(np.sqrt(0.5))
    if e == 2:
        return ((zr - zi) * h, (zr + zi) * h) if sign > 0 else ((zr + zi) * h, (zi - zr) * h)
    if e == 6:
        return ((zr + zi) * -h, (zr - zi) * h) if sign > 0 else ((zi - zr) * h, (zr + zi) * -h)
    c = float(np.cos(2 * np.pi * e / 16))
    s = float(sign * np.sin(2 * np.pi * e / 16))
    return (zr * c - zi * s, zr * s + zi * c)


def _dft16(x, sign):
    cols = [_dft4([x[n1 + 4 * n2] for n2 in range(4)], sign) for n1 in range(4)]
    out = [None] * 16
    for k2 in range(4):
        res = _dft4([_twiddle16(cols[n1][k2], n1 * k2, sign) for n1 in range(4)], sign)
        for k1 in range(4):
            out[k2 + 4 * k1] = res[k1]
    return out


def _kernel(ax_hbm, mem_ref, wq_hbm, wk_hbm, wv_hbm, wo_hbm, bx_hbm, wr_hbm, wi_hbm,
            wrn_ref, win_ref, fd_hbm, tab_ref, out_hbm,
            wqkv, wo, ax, ao, bx, wr, wi, fd, cm, y, xa, qa, h_ref, ob_ref, acc_ref,
            sem_w, sem_m, sem_o):
    qkv_u32 = [w.bitcast(U32) for w in (wq_hbm, wk_hbm, wv_hbm)]
    wo_u32 = wo_hbm.bitcast(U32)
    bx_u32 = bx_hbm.bitcast(U32)
    out_u32 = out_hbm.bitcast(U32)

    def bx_copy(c):
        return pltpu.make_async_copy(bx_u32.at[:, c, :], bx.at[c], sem_m.at[6 + c])

    def slab_copy(j, hp):
        return pltpu.make_async_copy(qkv_u32[j].at[:, hp, :], wqkv.at[j * 16 + hp + 1],
                                     sem_w.at[j * 16 + hp])

    def slab_wait(i):
        pltpu.make_async_copy(wqkv.at[i + 1], wqkv.at[i + 1], sem_w.at[i]).wait()

    def repair(i):
        for g in range(8):
            ev = wqkv[i + 1, pl.ds(g * 128, 64, stride=2), :]
            od = wqkv[i + 1, pl.ds(g * 128 + 1, 64, stride=2), :]
            wqkv[i, g * 64:(g + 1) * 64, :] = (ev & jnp.uint32(0xFFFF)) | (od << 16)
            wqkv[i, 512 + g * 64:512 + (g + 1) * 64, :] = (
                (ev >> 16) | (od & jnp.uint32(0xFFFF0000)))

    unroll = 4
    early = unroll + 1
    cp_fd = pltpu.make_async_copy(fd_hbm, fd, sem_m.at[0])

    def w_copies(c):
        return [pltpu.make_async_copy(
            src.at[pl.ds(0, 512)].bitcast(U32).at[:, pl.ds(pl.multiple_of(m1 * 128, 128), 128)],
            dst.at[m1], sem_m.at[2])
            for src, dst in ((wr_hbm, wr), (wi_hbm, wi)) for m1 in (2 * c, 2 * c + 1)]

    def wo_copy(n):
        return pltpu.make_async_copy(wo_u32.at[:, pl.ds(pl.multiple_of(n * 128, 128), 128)],
                                     wo.at[n], sem_m.at[3])

    cp_lo = pltpu.make_async_copy(ax_hbm.at[:, 0], ax.at[:, 0], sem_m.at[1])
    cp_hi0, cp_hi1 = (
        pltpu.make_async_copy(ax_hbm.at[segs, pl.ds(1, 3)], ax.at[segs, pl.ds(1, 3)], sem_m.at[k])
        for segs, k in ((pl.ds(0, early), 4), (pl.ds(early, _NSEG - early), 5)))
    cp_fd.start()
    for c in range(3):
        bx_copy(c).start()
    for cp in w_copies(0):
        cp.start()

    h2 = float(np.sqrt(0.5))

    def half(u, par):
        u = (u << 16) if par == 0 else (u & jnp.uint32(0xFFFF0000))
        return lax.bitcast_convert_type(u, F32)

    def s_matrix(a, carry):
        c0, s0 = tab_ref[0:128, 0:128], tab_ref[0:128, 128:256]
        rows = pl.ds(pl.multiple_of(128 + 8 * a, 8), 8)
        tc, ts = tab_ref[rows, 0:128][0:1], tab_ref[rows, 128:256][0:1]
        cc, ss = c0 * tc - s0 * ts, c0 * ts + s0 * tc
        cm[a, 0:128, 0:128] = cc.astype(BF16)
        cm[a, 0:128, 128:256] = ss.astype(BF16)
        cm[a, 128:256, 0:128] = (-ss).astype(BF16)
        cm[a, 128:256, 128:256] = cc.astype(BF16)
        return carry

    lax.fori_loop(0, 16, s_matrix, 0)
    cp_fd.wait()

    def forward(c, carry):
        @pl.when(c < 5)
        def _():
            bx_copy(c + 3).start()

        @pl.when(c < 7)
        def _():
            for cp in w_copies(c + 1):
                cp.start()

        @pl.when(c >= 5)
        def _():
            slab_copy(0, c - 5).start()

        @pl.when(c == 5)
        def _():
            cp_lo.start()

        bx_copy(c).wait()
        for par in range(2):
            a = 2 * c + par
            x = [half(bx[c, :, t * 128:(t + 1) * 128], par) for t in range(8)]
            e0, e1, e2, e3 = x[0] + x[4], x[0] - x[4], x[2] + x[6], x[2] - x[6]
            o0, o1, o2, o3 = x[1] + x[5], x[1] - x[5], x[3] + x[7], x[3] - x[7]
            ee, oo = e0 + e2, o0 + o2
            p, q = (o1 - o3) * h2, (o1 + o3) * h2
            ts = ((e1 + p, -(e3 + q)), (e0 - e2, o2 - o0), (e1 - p, e3 - q))
            re, im = [], []
            for g in range(3):
                t = jnp.concatenate([ts[g][0].astype(BF16), ts[g][1].astype(BF16)], axis=1)
                r = lax.dot_general(fd[g * 256:(g + 1) * 256, :], t, _NT,
                                    preferred_element_type=F32)
                re.append(r[0:128])
                im.append(r[128:256])
            r = lax.dot_general(fd[768:896, 0:128], (ee - oo).astype(BF16), _NT,
                                preferred_element_type=F32)
            re.append(r[0:64])
            im.append(r[64:128])
            r = lax.dot_general(fd[896:1040, 0:128], (ee + oo).astype(BF16), _NT,
                                preferred_element_type=F32)
            re.append(r[0:72])
            im.append(r[72:144])
            for r0, r1, g0, g1 in ((0, 256, 0, 2), (256, _KR, 2, 5)):
                u = jnp.concatenate([jnp.concatenate(re[g0:g1], axis=0),
                                     jnp.concatenate(im[g0:g1], axis=0)], axis=1)
                y[a, r0:r1, :] = jnp.dot(u, cm[a], preferred_element_type=F32)
        return carry

    lax.fori_loop(0, 8, forward, 0)
    slab_copy(0, 3).start()
    for c in range(8):
        for cp in w_copies(c):
            cp.wait()

    def spectral(rows, filt):
        xf = _dft16([(y[a, rows, 0:128], y[a, rows, 128:256]) for a in range(16)], -1)
        v = []
        for m1 in range(16):
            (xr, xi), (fr, fi) = xf[m1], filt(m1)
            v.append((xr * fr - xi * fi, xr * fi + xi * fr))
        res = _dft16(v, +1)
        for a in range(16):
            y[a, rows, 0:128] = res[a][0]
            y[a, rows, 128:256] = res[a][1]

    cp_lo.wait()
    for g in range(8):
        xa[g * 64:(g + 1) * 64, :] = (
            ax[g * 8:(g + 1) * 8, 0, :, :].astype(F32).reshape(64, _D))
    slab_wait(0)
    repair(0)

    def middle(i, carry):
        @pl.when(i < 12)
        def _():
            slab_copy(0, i + 4).start()

        slab_copy(1, i).start()

        @pl.when(i % 4 != 3)
        def _():
            slab_copy(2, i - i // 4).start()

        slab_wait(i + 1)
        repair(i + 1)
        c = i // 4
        for par in range(2):
            w = pltpu.bitcast(wqkv[i, par * 512:(par + 1) * 512, :], BF16)
            blk = _RES.index(par)
            for cc in range(1, 4):
                blk = jnp.where(c == cc, _RES.index(2 * cc + par), blk)
            for k in range(2):
                qa[2 * i + par, k * 256:(k + 1) * 256] = jnp.dot(
                    xa[k * 256:(k + 1) * 256], w, preferred_element_type=F32)
                jg = 2 * (i % 4) + k
                w_rows = pl.ds(jg * 32 + c, 8, stride=4)
                spectral(pl.ds(pl.multiple_of(blk * 64 + jg * 8, 8), 8),
                         lambda m1: (half(wr[m1, w_rows, :], par), half(wi[m1, w_rows, :], par)))
        return carry

    lax.fori_loop(0, 16, middle, 0)
    spectral(pl.ds(512, 8),
             lambda m1: tuple(jnp.broadcast_to(w[0:1, m1 * 128:(m1 + 1) * 128].astype(F32), (8, 128))
                             for w in (wrn_ref, win_ref)))

    sign = jnp.where(lax.broadcasted_iota(jnp.int32, (128, 256), 0) % 2 == 0, 1.0, -1.0)

    def b_out_copy(c):
        return pltpu.make_async_copy(bx.at[c], out_u32.at[:, c, pl.ds(_D, _D)], sem_o.at[0])

    def inverse(c, carry):
        @pl.when(c < 4)
        def _():
            wo_copy(2 * c).start()
            wo_copy(2 * c + 1).start()

        slab_wait(17 + 2 * c)
        slab_wait(18 + 2 * c)
        zs = {}
        for par in range(2):
            a = 2 * c + par
            for g in range(4):
                z = lax.dot_general(cm[a], y[a, g * 128:(g + 1) * 128, :].astype(BF16), _NT,
                                    preferred_element_type=F32)
                zr, zi = z[0:128], z[128:256]
                if g < 3:
                    zs[par, g] = jnp.concatenate([zr, zi], axis=1).astype(BF16)
                else:
                    low = lax.broadcasted_iota(jnp.int32, (128, 128), 1) < 64
                    zs[par, 3] = jnp.where(low, zr, pltpu.roll(zi, 64, 1)).astype(BF16)
                    zs[par, 4] = jnp.where(low, pltpu.roll(zr, 64, 1), zi).astype(BF16)
            zs[par, 5] = lax.dot_general(
                cm[a, 0:128, :], (y[a, 512:513, :] * sign).astype(BF16), _NT,
                preferred_element_type=F32)
        outs = []
        for par in range(2):
            qs = []
            for g in range(3):
                r = jnp.dot(zs[par, g], fd[g * 256:(g + 1) * 256, :],
                            preferred_element_type=F32)
                qs.append((r[:, 0:128], r[:, 128:256]))
            (q1r, q1i), (q2r, q2i), (q3r, q3i) = qs
            r4 = jnp.dot(zs[par, 3], fd[768:896, 0:128], preferred_element_type=F32)
            r0 = jnp.dot(zs[par, 4], fd[768:896, 128:256],
                         preferred_element_type=F32) + zs[par, 5]
            ee, oo = r0 + r4, r0 - r4
            e0, e2, o0, o2 = ee + q2r, ee - q2r, oo - q2i, oo + q2i
            e1, e3 = q1r + q3r, q3i - q1i
            p, q = (q1r - q3r) * h2, (q1i + q3i) * h2
            o1, o3 = p - q, -(p + q)
            cols = (e0 + e1, o0 + o1, e2 + e3, o2 + o3, e0 - e1, o0 - o1, e2 - e3, o2 - o3)
            outs.append([lax.bitcast_convert_type(v.astype(BF16).astype(F32), U32)
                         for v in cols])
        for t in range(8):
            bx[c, :, t * 128:(t + 1) * 128] = (outs[0][t] >> 16) | outs[1][t]
        repair(17 + 2 * c)
        repair(18 + 2 * c)
        return carry

    for hp in range(12, 16):
        slab_copy(2, hp).start()
    cp_hi0.start()
    lax.fori_loop(0, 8, inverse, 0)

    def last_slabs(i, carry):
        slab_wait(i)
        repair(i)
        return carry

    lax.fori_loop(33, 48, last_slabs, 0)
    for hd in range(_NK):
        w = pltpu.bitcast(wqkv[16 + hd // 2, (hd % 2) * 512:(hd % 2 + 1) * 512, :], BF16)
        qa[_H + hd] = jnp.dot(xa[...], w, preferred_element_type=F32)
    cp_hi0.wait()
    for n in range(8):
        wo_copy(n).wait()
    cp_hi1.start()

    def position(i):
        return jnp.where(i < 8, i + _M, jnp.where(i < 8 + _M, i - 8, i))

    qi = position(lax.broadcasted_iota(jnp.int32, (_L, _L), 0))
    ki = position(lax.broadcasted_iota(jnp.int32, (_L, _L), 1))
    mask = (qi < _M) | (qi >= ki)
    scale = 128 ** -0.5
    group, skew, lag, slag, order = 8, 2, 2, 1, 'kqsvop'
    n_group = _H // group

    def load_tokens(s):
        for k, r0 in enumerate((0, 16, 24, 32)):
            h_ref[r0:r0 + 8, :] = ax[s, k].astype(F32)

    h_ref[8:16, :] = mem_ref[...].astype(F32)
    load_tokens(0)

    def a_out_copy(s):
        rows = pl.ds(2 * s, 2)
        return pltpu.make_async_copy(ao.at[rows], out_hbm.at[rows, :, pl.ds(0, _D)],
                                     sem_o.at[1])

    def step(s):
        st = {}

        def proj(j, hd):
            w = wqkv[j * 16 + hd // 2, (hd % 2) * 512:(hd % 2 + 1) * 512, :]
            hoisted = j * _H + hd < _H + _NK
            r = jnp.dot(h_ref[(8 if hoisted else 0):_L, :], pltpu.bitcast(w, BF16),
                        preferred_element_type=F32)
            if hoisted:
                r = jnp.concatenate(
                    [qa[j * _H + hd, pl.ds(pl.multiple_of(s * 8, 8), 8), :], r], axis=0)
            st[j, hd] = r

        def scores(hd):
            sc = lax.dot_general(st[0, hd], st[1, hd], _NT, preferred_element_type=F32) * scale
            sc = jnp.where(mask, sc, -1000000000.0)
            p = jnp.exp(sc - jnp.max(sc, axis=1, keepdims=True))
            st['p', hd] = p
            st['l', hd] = 1.0 / jnp.sum(p, axis=1, keepdims=True)

        def pv(hd):
            o = jnp.dot(st['p', hd], st[2, hd], preferred_element_type=F32)
            ob_ref[:, hd * 128:(hd + 1) * 128] = o * st['l', hd]

        def w_out(g, n):
            lanes = slice(n * 128, (n + 1) * 128)
            w = wo[n, g * group * 64:(g + 1) * group * 64, :]
            r = jnp.dot(ob_ref[:, g * group * 128:(g + 1) * group * 128],
                        pltpu.bitcast(w, BF16), preferred_element_type=F32)
            if g > 0:
                r = r + acc_ref[:, lanes]
            if g < n_group - 1:
                acc_ref[:, lanes] = r
            else:
                h_ref[8:16, lanes] = r[8:16].astype(BF16).astype(F32)
                ao[2 * s, :, lanes] = jnp.concatenate([r[0:8], r[16:24]], axis=0).astype(BF16)
                ao[2 * s + 1, :, lanes] = r[24:40].astype(BF16)

        def next_x():
            load_tokens(jnp.minimum(s + 1, _NSEG - 1))

        ops, pending = [], []
        for t in range(_H + skew + lag + slag):
            for what in order:
                if what == 'q' and t < _H:
                    ops.append((proj, 0, t))
                if what == 'k' and t < _H:
                    ops.append((proj, 1, t))
                if what == 's' and 0 <= t - slag < _H:
                    ops.append((scores, t - slag))
                if what == 'o' and pending:
                    ops.append(pending.pop(0))
                if what == 'v' and 0 <= t - skew < _H:
                    ops.append((proj, 2, t - skew))
                    if t - skew == _H - 1:
                        ops.append((next_x,))
                hd = t - skew - lag
                if what == 'p' and 0 <= hd < _H:
                    if hd == _H - 1:
                        ops += pending
                        pending = []
                    ops.append((pv, hd))
                    if hd % group == group - 1:
                        pending += [(w_out, hd // group, n) for n in range(8)]
        ops += pending
        for op in ops:
            op[0](*op[1:])
        a_out_copy(s).start()

    def segments(part, carry):
        def steps(i, c):
            for k in range(unroll):
                step(unroll * i + k)
            return c

        lax.fori_loop(part, 1 + part * (_NSEG // unroll - 1), steps, 0)

        @pl.when(part == 0)
        def _():
            cp_hi1.wait()
            for c in range(8):
                b_out_copy(c).start()

        return carry

    lax.fori_loop(0, 2, segments, 0)

    def drain_b(a, carry):
        b_out_copy(a).wait()
        return carry

    def drain_a(s, carry):
        a_out_copy(s).wait()
        return carry

    lax.fori_loop(0, 8, drain_b, 0)
    lax.fori_loop(0, _NSEG, drain_a, 0)


@jax.jit
def _run(A_x, A_mem0, A_Wq, A_Wk, A_Wv, A_Wo, B_x, B_w_r, B_w_i):
    hbm = pl.BlockSpec(memory_space=pltpu.HBM)
    vmem = pl.BlockSpec(memory_space=pltpu.VMEM)
    nyquist = pl.BlockSpec((16, _S), lambda i: (512 // 16, 0))
    wr, wi = B_w_r.T, B_w_i.T
    out = pl.pallas_call(
        _kernel,
        grid=(1,),
        out_shape=jax.ShapeDtypeStruct((128, 16, 2 * _D), BF16),
        in_specs=[hbm, vmem, hbm, hbm, hbm, hbm, hbm, hbm, hbm, nyquist, nyquist, hbm, vmem],
        out_specs=hbm,
        scratch_shapes=[
            pltpu.VMEM((49, 1024, 128), U32),
            pltpu.VMEM((8, 2048, 128), U32),
            pltpu.VMEM((_NSEG, 4, 8, _D), BF16),
            pltpu.VMEM((128, 16, _D), BF16),
            pltpu.VMEM((8, 128, _D), U32),
            pltpu.VMEM((16, 256, 128), U32),
            pltpu.VMEM((16, 256, 128), U32),
            pltpu.VMEM((1040, 256), BF16),
            pltpu.VMEM((16, 256, 256), BF16),
            pltpu.VMEM((16, _KR, 256), F32),
            pltpu.VMEM((_NSEG * 8, _D), F32),
            pltpu.VMEM((_H + _NK, _NSEG * 8, 128), F32),
            pltpu.VMEM((_L, _D), F32),
            pltpu.VMEM((_L, _H * 128), F32),
            pltpu.VMEM((_L, _D), F32),
            pltpu.SemaphoreType.DMA((48,)),
            pltpu.SemaphoreType.DMA((14,)),
            pltpu.SemaphoreType.DMA((2,)),
        ],
        compiler_params=pltpu.CompilerParams(vmem_limit_bytes=100 * 1024 * 1024),
    )(A_x.reshape(_NSEG, 4, 8, _D), A_mem0.reshape(_M, _D), A_Wq, A_Wk, A_Wv,
      A_Wo.reshape(_H * 128, _D), B_x.reshape(128, 16, _D), wr, wi, wr, wi, *_CONSTS)
    return out.reshape(1, _S, 2 * _D)


def pallas_concat_heads__memory_aug_recurrent_mem_tr__spectral_gfnet__prompt_kernel(
    A_x, A_mem0, A_Wq, A_Wk, A_Wv, A_Wo, A_seg_len, B_x, B_w_r, B_w_i,
):
    assert int(A_seg_len) == _SEG
    return _run(A_x, A_mem0, A_Wq, A_Wk, A_Wv, A_Wo, B_x, B_w_r, B_w_i)
```
